```python
import os as _os
_os.environ.setdefault("JAX_PLATFORMS", "cpu")
import jax
import jax.numpy as jnp

def _softmax(x, axis=-1):
    return jax.nn.softmax(x, axis=axis)
def _gelu(x):
    return jax.nn.gelu(x, approximate=True)
def _silu(x):
    return jax.nn.silu(x)
def _sigmoid(x):
    return jax.nn.sigmoid(x)
def _layernorm(x, axis=-1, eps=1e-5):
    m = jnp.mean(x, axis=axis, keepdims=True)
    v = jnp.var(x, axis=axis, keepdims=True)
    return (x - m) / jnp.sqrt(v + eps)
def _scatter_add(tgt, idx, src, axis=0):
    return tgt.at[idx].add(src)
def _segment_sum(src, seg, n):
    return jax.ops.segment_sum(src, seg, n)
class _Rng:
    def __init__(self, key):
        self._k = key
    def _next(self):
        self._k, sub = jax.random.split(self._k)
        return sub
    def normal(self, shape):
        return jax.random.normal(self._next(), shape, dtype=jnp.bfloat16)
    def randint(self, lo, hi, shape):
        return jax.random.randint(self._next(), shape, lo, hi, dtype=jnp.int32)
    def uniform(self, shape, lo=0.0, hi=1.0):
        return jax.random.uniform(self._next(), shape, jnp.bfloat16, lo, hi)
    def permutation(self, n):
        return jax.random.permutation(self._next(), n)


kernel_name = 'interleave_layers__ssm_conv_h3__geglu_ffn__prompt'

def setup_inputs():
    _rng = _Rng(jax.random.key(int.from_bytes(__import__("os").urandom(4), "little")))
    _w = (lambda a: (lambda t: t.astype(jnp.bfloat16) if jnp.issubdtype(t.dtype, jnp.floating) else t)(jnp.asarray(a)))
    def _A_setup():
        B, S, D = 1, 2048, 448
        ks = 4
        return {
            "q": _w((lambda *s: _rng.normal(s) * 0.05)(B, S, D)),
            "k": _w((lambda *s: _rng.normal(s) * 0.8)(B, S, D)),
            "v": _w((lambda *s: _rng.normal(s) * 0.8)(B, S, D)),
            "shift_k": _w((lambda *s: _rng.normal(s) * 0.8)(D, ks) * 0.5),
            "ssm_k": _w((lambda *s: _rng.normal(s) * 0.8)(D, S) * (1.0 / S ** 0.5)),
            "ssm_D": _w((lambda *s: _rng.normal(s) * 0.8)(D)),
        }
    _A_in = _A_setup()

    def _B_setup():
        B, S, D, F = 1, 2048, 448, 1792
        return {
            "x": _w((lambda *s: _rng.normal(s) * 0.05)(B, S, D)),
            "w_gate": _w((lambda *s: _rng.normal(s) * 0.1)(D, F)),
            "w_up": _w((lambda *s: _rng.normal(s) * 0.1)(D, F)),
            "w_down": _w((lambda *s: _rng.normal(s) * 0.1)(F, D)),
        }
    _B_in = _B_setup()

    return {
        "A_q": _A_in["q"],
        "A_k": _A_in["k"],
        "A_v": _A_in["v"],
        "A_shift_k": _A_in["shift_k"],
        "A_ssm_k": _A_in["ssm_k"],
        "A_ssm_D": _A_in["ssm_D"],
        "B_x": _B_in["x"],
        "B_w_gate": _B_in["w_gate"],
        "B_w_up": _B_in["w_up"],
        "B_w_down": _B_in["w_down"],
    }

def reference(A_q, A_k, A_v, A_shift_k, A_ssm_k, A_ssm_D, B_x, B_w_gate, B_w_up, B_w_down):
    def _A_ref(q, k, v, shift_k, ssm_k, ssm_D):
        B, S, D = q.shape
        ks = shift_k.shape[-1]
        k_pad = jnp.pad(k, ((0, 0), (ks - 1, 0), (0, 0)))
        k_shift = jnp.zeros_like(k)
        for t in range(ks):
            k_shift = k_shift + k_pad[:, t:t + S, :] * shift_k[:, ks - 1 - t][None, None, :]
        kv = k_shift * v
        L = 2 * S
        kv_pad = jnp.pad(kv, ((0, 0), (0, S), (0, 0)))
        kf_pad = jnp.pad(ssm_k, ((0, 0), (0, S)))
        kv_f = (lambda x, axes=(-2,-1): jnp.fft.rfft2(x.astype(jnp.float32), axes=axes))(kv_pad[:, None, :, :], axes=(1, 2))
        kf_f = (lambda x, axes=(-2,-1): jnp.fft.rfft2(x.astype(jnp.float32), axes=axes))(kf_pad[:, None, :], axes=(1, 2))
        kf_f = (lambda x, *d: x.transpose(*d))(kf_f, 1, 2, 0)
        y_f = kv_f * kf_f[None, :, :, :]
        y = (lambda x, s, axes=(-2,-1): jnp.fft.irfft2(x, s=s, axes=axes).astype(jnp.bfloat16))(y_f, (1, L), axes=(1, 2))[:, 0, :S, :]
        y = y + kv * ssm_D[None, None, :]
        return q * y

    def _B_ref(x, w_gate, w_up, w_down):
        return (_gelu(x @ w_gate) * (x @ w_up)) @ w_down

    x = A_q
    x = x + _A_ref(_layernorm(x, axis=-1), A_k, A_v, A_shift_k, A_ssm_k, A_ssm_D)
    x = x + _B_ref(_layernorm(x, axis=-1), B_w_gate, B_w_up, B_w_down)
    x = x + _A_ref(_layernorm(x, axis=-1), A_k, A_v, A_shift_k, A_ssm_k, A_ssm_D)
    x = x + _B_ref(_layernorm(x, axis=-1), B_w_gate, B_w_up, B_w_down)
    return x
```

```python
import functools
import numpy as np
import jax
import jax.numpy as jnp
from jax import lax
import jax.experimental.pallas as pl
import jax.experimental.pallas.tpu as pltpu

B = 128
PB = 2
TM = PB * B
GELU_C = 0.7978845608028654
EPS = 1e-5
F32 = jnp.float32
BF16 = jnp.bfloat16


def _dft_tables():
    n = np.arange(B)[:, None]
    k = np.arange(B)[None, :]
    ang = 2.0 * np.pi * (((2 * k + 1) * n) % (4 * B)) / (4 * B)
    ft = np.concatenate([np.cos(ang), -np.sin(ang)], axis=1)
    return ft.astype(np.float32), (ft.T / B).astype(np.float32)


def _stat_terms(x, y, cb):
    a = x - cb
    ay = a * y
    return a, a * a, ay, a * ay, ay * y, ay * ay


def _rsqrt_valu(x):
    i = lax.bitcast_convert_type(x, jnp.int32)
    y = lax.bitcast_convert_type(jnp.int32(0x5F3759DF) - lax.shift_right_logical(i, jnp.int32(1)), F32)
    hx = 0.5 * x
    for _ in range(4):
        y = y * (1.5 - hx * y * y)
    return y


def _stats(c, sums, y1, y2, d, rsqrt=lax.rsqrt):
    s1, s2, t1, t2, v1, v2 = [jnp.sum(t, axis=0, keepdims=True) for t in sums]
    inv = 1.0 / d
    m = s1 * inv
    e2 = s2 * inv
    r = rsqrt(jnp.maximum(e2 - m * m, 0.0) + EPS)
    mb = m + r * (t1 - m * y1) * inv
    eb = e2 + (2.0 * inv) * r * (t2 - m * t1) + (r * r * inv) * (v2 - 2.0 * m * v1 + m * m * y2)
    r3 = rsqrt(jnp.maximum(eb - mb * mb, 0.0) + EPS)
    return c + m, r, c + mb, r3


def _acc(accs, vals):
    return list(vals) if accs is None else [a + v for a, v in zip(accs, vals)]


def _gelu(x):
    inner = x * (GELU_C + (GELU_C * 0.044715) * (x * x))
    return (0.5 * x) * (1.0 + jnp.tanh(inner))


def _pack(x):
    return pltpu.bitcast(x, jnp.uint32)


def _unpack(x):
    return pltpu.bitcast(x, BF16)


_TN = (((0,), (0,)), ((), ()))


def _kernel(q_ref, k_ref, v_ref, h_ref, k0_ref, v0_ref, h0_ref, sk_ref, d_ref, ft_ref, fi_ref,
            wg_ref, wu_ref, wdt_ref,
            o_ref,
            ug_ref, kv_ref, yf_ref, xn_ref, ys_ref, wt_ref, wd_ref,
            *, D, F, NB, CH, JG, KS, MODE, AG):
    s = pl.program_id(0)
    P = NB * PB
    PAD = P - 1
    UBASE = PAD
    HBASE = PAD + P + PB
    ZP = HBASE + P + PB
    KVD, YST, CB, FENCE, YY, X1, X2, X3 = ZP + 1, ZP + 2, ZP + 3, ZP + 6, ZP + 7, ZP + 8, ZP + 9, ZP + 10
    zd = jnp.minimum(s, 0)
    lo, hi = slice(0, B), slice(B, 2 * B)
    starts = [sum(CH[:i]) for i in range(len(CH))]
    NC = len(CH)

    def init():
        rows = lax.broadcasted_iota(jnp.int32, (16, D), 0)
        a = jnp.zeros((16, D), F32)
        skf = sk_ref[...].astype(F32)
        for j in range(KS):
            a = jnp.where(rows == j, jnp.broadcast_to(skf[j:j + 1, :], (16, D)), a)
        a = jnp.where(rows == KS, jnp.broadcast_to(d_ref[...].astype(F32), (16, D)), a)
        ab = a.astype(BF16)
        er = lax.broadcasted_iota(jnp.int32, (16, 2 * B), 0)
        ec = lax.broadcasted_iota(jnp.int32, (16, 2 * B), 1) // B
        for t in range(3):
            e = jnp.where(er == ec + 2 * t, 1.0, 0.0).astype(BF16)
            ug_ref[CB + t] = lax.dot_general(ab, e, _TN, preferred_element_type=F32)
        ug_ref[ZP] = jnp.zeros((D, 2 * B), F32)
        ug_ref[0:PAD] = jnp.zeros((PAD, D, 2 * B), F32)

    def prep_weights():
        for c in range(F // 256):
            cs = slice(c * 256, (c + 1) * 256)
            gt = _pack(wg_ref[:, cs].T)
            ut = _pack(wu_ref[:, cs].T)
            for i in range(16):
                r0 = c * 256 + i * 16
                wt_ref[r0:r0 + 8, :] = gt[i * 8:(i + 1) * 8]
                wt_ref[r0 + 8:r0 + 16, :] = ut[i * 8:(i + 1) * 8]
            wd_ref[:, cs] = _pack(wdt_ref[:, cs])

    def kv_full(kr, vr):
        lane = lax.broadcasted_iota(jnp.int32, (D, B), 1)
        taps = [ug_ref[CB + j // 2, :, (lo, hi)[j % 2]] for j in range(KS)]
        dcol = ug_ref[CB + 2, :, lo]
        kp = ug_ref[CB + 2, :, hi]
        for p in range(PB):
            ps = slice(p * B, (p + 1) * B)
            kc = kr[:, ps].astype(F32)
            acc = kc * taps[0]
            for j in range(1, KS):
                sh = jnp.where(lane < j, pltpu.roll(kp, j, 1), pltpu.roll(kc, j, 1))
                acc = acc + sh * taps[j]
            kvb = (acc * vr[:, ps].astype(F32)).astype(BF16)
            kv_ref[:, ps] = _pack(kvb)
            ug_ref[KVD, :, ps] = kvb.astype(F32) * dcol
            kp = kc
        ug_ref[CB + 2, :, hi] = kp

    def kv_half(g, p, kr, vr):
        rs = slice(g * 16, (g + 1) * 16)
        ps = slice(p * B, (p + 1) * B)
        lane = lax.broadcasted_iota(jnp.int32, (16, B), 1)
        taps = [ug_ref[CB + zd + j // 2, rs, (lo, hi)[j % 2]] for j in range(KS)]
        dcol = ug_ref[CB + 2 + zd, rs, lo]
        kp = ug_ref[CB + 2 + zd, rs, hi] if p == 0 else kr[rs, (p - 1) * B:p * B].astype(F32)
        kc = kr[rs, ps].astype(F32)
        acc = kc * taps[0]
        for j in range(1, KS):
            sh = jnp.where(lane < j, pltpu.roll(kp, j, 1), pltpu.roll(kc, j, 1))
            acc = acc + sh * taps[j]
        kvb = (acc * vr[rs, ps].astype(F32)).astype(BF16)
        kv_ref[g * 8:(g + 1) * 8, ps] = _pack(kvb)
        ug_ref[KVD, rs, ps] = kvb.astype(F32) * dcol
        if p == PB - 1:
            ug_ref[CB + 2, rs, hi] = kc

    def fwd_h(hr, blk):
        p0 = jnp.minimum(blk, NB) * PB
        for p in range(PB):
            ug_ref[HBASE + p0 + p] = jnp.dot(hr[:, p * B:(p + 1) * B], ft_ref[...], preferred_element_type=F32)

    def fwd_u(blk):
        p0 = jnp.minimum(blk, NB) * PB
        for p in range(PB):
            ug_ref[UBASE + p0 + p] = jnp.dot(_unpack(kv_ref[:, p * B:(p + 1) * B]), ft_ref[...], preferred_element_type=F32)

    def mac_rows(r, nj, blk):
        p0 = blk * PB
        gmax = p0 + PB - 1
        rs = slice(r * 8, (r + 1) * 8)
        sgn = jnp.where(lax.broadcasted_iota(jnp.int32, (8, B), 1) % 2 == 0, 1.0, -1.0)
        ar = [None] * PB
        ai = [None] * PB
        us = {}
        for j in range(nj):
            gj = HBASE + jnp.minimum(j, gmax)
            gr = ug_ref[gj, rs, lo]
            gi = ug_ref[gj, rs, hi]
            for p in range(PB):
                off = p - j
                if off not in us:
                    us[off] = (ug_ref[UBASE + p0 + off, rs, lo], ug_ref[UBASE + p0 + off, rs, hi])
                ur, ui = us[off]
                tr = ur * gr - ui * gi
                ti = ur * gi + ui * gr
                ar[p] = tr if ar[p] is None else ar[p] + tr
                ai[p] = ti if ai[p] is None else ai[p] + ti
            if (j + 1) % JG == 0 and j + 1 < nj:
                for p in range(PB):
                    ug_ref[FENCE, p * 8:(p + 1) * 8, lo] = ar[p]
                    ug_ref[FENCE, p * 8:(p + 1) * 8, hi] = ai[p]
        zr, zi = ug_ref[ZP + zd, rs, lo], ug_ref[ZP + zd, rs, hi]
        out = []
        for p in range(PB):
            out.append((ar[p] - sgn * zi, ai[p] + sgn * zr))
            zr, zi = ar[p], ai[p]
        ug_ref[ZP, rs, lo] = zr
        ug_ref[ZP, rs, hi] = zi
        ug_ref[FENCE, 0:8, lo] = out[0][0]
        ug_ref[FENCE, 0:8, hi] = out[0][1]
        return out

    def mac_group(g, nj, blk):
        res = [mac_rows(2 * g + i, nj, blk) for i in range(2)]
        rs = slice(g * 8, (g + 1) * 8)
        for p in range(PB):
            yf_ref[p, rs, lo] = _pack(jnp.concatenate([x[p][0] for x in res], axis=0).astype(BF16))
            yf_ref[p, rs, hi] = _pack(jnp.concatenate([x[p][1] for x in res], axis=0).astype(BF16))

    def inv_dot():
        for p in range(PB):
            ps = slice(p * B, (p + 1) * B)
            ug_ref[YST, :, ps] = jnp.dot(_unpack(yf_ref[p]), fi_ref[...], preferred_element_type=F32) + ug_ref[KVD, :, ps]

    def side_post(z, old, kr, vr):
        c = q_ref[0:16, :].astype(F32)[0:1]
        cb = jnp.broadcast_to(c, (8, TM))
        accs = None
        for g in range(D // 16):
            rs = slice(g * 16, (g + 1) * 16)
            if old is not None:
                x = ug_ref[X2 + z, rs, :]
                ug_ref[X3, rs, :] = x + (x - old[0]) * old[1] * ug_ref[YY + z, rs, :]
            x = q_ref[rs, :].astype(F32)
            y = ug_ref[YST + z, rs, :]
            for i in range(2):
                yi = y[i * 8:(i + 1) * 8]
                accs = _acc(accs, _stat_terms(x[i * 8:(i + 1) * 8], yi, cb) + (yi, yi * yi))
            if kr is not None:
                kv_half(g, 0, kr, vr)
        y1 = jnp.sum(accs[6], axis=0, keepdims=True)
        y2 = jnp.sum(accs[7], axis=0, keepdims=True)
        ys_ref[0:1, :] = y1
        ys_ref[8:9, :] = y2
        mu, r, mu3, r3 = _stats(c, accs[:6], y1, y2, D, _rsqrt_valu)
        for g in range(D // 16):
            rs = slice(g * 16, (g + 1) * 16)
            x = q_ref[rs, :].astype(F32)
            y = ug_ref[YST + z, rs, :]
            xo = x + (x - mu) * r * y
            xn = (xo - mu3) * r3
            xn_ref[g * 8:(g + 1) * 8, :] = _pack(xn.astype(BF16))
            ug_ref[YY, rs, :] = y
            ug_ref[X1, rs, :] = xo
            if kr is not None:
                ug_ref[FENCE, 0:8, lo] = xn[8:16, B:2 * B]
                kv_half(g, 1, kr, vr)

    def gu(c, xn):
        f0, fc = starts[c], CH[c]
        return jnp.dot(_unpack(wt_ref[f0:f0 + fc, :]), xn, preferred_element_type=F32)

    def act(c, r):
        hs = [(_gelu(r[32 * i:32 * i + 16]) * r[32 * i + 16:32 * i + 32]).astype(BF16) for i in range(CH[c] // 16)]
        return jnp.concatenate(hs, axis=0)

    def dn(c, hh, acc):
        f0, fc = starts[c], CH[c]
        return jnp.dot(_unpack(wd_ref[:, f0:f0 + fc]), hh, preferred_element_type=F32) + acc

    def mlp(xn, side, first_acc, res_slot, res_chunk):
        raws = [gu(0, xn), gu(1, xn)]
        side(raws)
        acc = None
        for c in range(NC):
            if 1 <= c < NC - 1:
                raws.append(gu(c + 1, xn))
            acc = dn(c, act(c, raws[c]), first_acc() if c == 0 else acc)
            if c == res_chunk:
                acc = acc + ug_ref[res_slot]
        return acc

    @pl.when(s == 0)
    def _():
        init()
        ug_ref[CB + 2, :, hi] = jnp.zeros((D, B), F32)
        kv_full(k0_ref, v0_ref)
        fwd_h(h0_ref, s)
        fwd_u(s)
        for g in range(D // 16):
            mac_group(g, PB, s)
        inv_dot()
        side_post(0, None, None, None)
        kv_full(k_ref, v_ref)
        fwd_h(h_ref, s + 1)
        fwd_u(s + 1)
        prep_weights()

    @pl.when(s > 0)
    def _():
        def side1(raws):
            n0, n1 = raws[0].shape[0], raws[1].shape[0]
            anchors = {0: raws[0][0:8, lo], AG[0]: raws[0][n0 - 8:n0, lo], AG[1]: raws[0][n0 - 8:n0, hi],
                       AG[2]: raws[1][n1 - 8:n1, lo], AG[3]: raws[1][n1 - 8:n1, hi]}
            for g in range(D // 16):
                if g in anchors:
                    ug_ref[FENCE, 0:8, lo] = anchors[g]
                mac_group(g, P, s)

        x2 = mlp(_unpack(xn_ref[...]), side1, lambda: ug_ref[X1], None, None)
        inv_dot()
        ug_ref[X2] = x2
        st = []
        for p in range(PB):
            ps = slice(p * B, (p + 1) * B)
            c = x2[0:1, ps]
            cb = jnp.broadcast_to(c, (8, B))
            accs = None
            for i in range(D // 8):
                accs = _acc(accs, _stat_terms(x2[i * 8:(i + 1) * 8, ps], ug_ref[YY, i * 8:(i + 1) * 8, ps], cb))
            st.append(_stats(c, accs, ys_ref[0:1, ps], ys_ref[8:9, ps], D))
        xn3 = []
        for p in range(PB):
            ps = slice(p * B, (p + 1) * B)
            mu, r, mu3, r3 = st[p]
            x2r = ug_ref[X2 + (zd if (p > 0 or MODE & 1) else 0), :, ps]
            xn3.append(((x2r + (x2r - mu) * r * ug_ref[YY, :, ps] - mu3) * r3).astype(BF16))
        old = [jnp.concatenate([st[p][i] for p in range(PB)], axis=1) for i in range(2)]

        def side2(raws):
            n0 = raws[0].shape[0]
            ug_ref[FENCE, 0:8, lo] = raws[0][n0 // 2 - 8:n0 // 2, hi]
            side_post(zd, old, k_ref, v_ref)

        x4 = mlp(jnp.concatenate(xn3, axis=1), side2, lambda: jnp.zeros((D, TM), F32), X3, NC - 2)
        fwd_h(h_ref, s + 1)
        fwd_u(s + 1)
        o_ref[...] = x4.astype(o_ref.dtype)


@jax.jit
def pallas_interleave_layers__ssm_conv_h3__geglu_ffn__prompt_kernel(
        A_q, A_k, A_v, A_shift_k, A_ssm_k, A_ssm_D, B_x, B_w_gate, B_w_up, B_w_down):
    CH = (512, 512, 512, 256)
    JG, MODE, A0, A1, A2, A3 = 4, 0, 6, 10, 14, 99
    _, S, D = A_q.shape
    F = B_w_gate.shape[1]
    KS = A_shift_k.shape[1]
    NB = S // TM
    P = S // B
    ft, fi = _dft_tables()
    ft = jnp.asarray(ft, BF16)
    fi = jnp.asarray(fi, BF16)
    qT = jnp.swapaxes(A_q, 1, 2).reshape(D, S)
    kT = jnp.swapaxes(A_k, 1, 2).reshape(D, S)
    vT = jnp.swapaxes(A_v, 1, 2).reshape(D, S)
    cur = pl.BlockSpec((D, TM), lambda s: (0, jnp.minimum(s, NB - 1)))
    nxt = pl.BlockSpec((D, TM), lambda s: (0, jnp.minimum(s + 1, NB - 1)))
    first = pl.BlockSpec((D, TM), lambda s: (0, 0))
    full = lambda shape: pl.BlockSpec(shape, lambda s: (0,) * len(shape))
    oT = pl.pallas_call(
        functools.partial(_kernel, D=D, F=F, NB=NB, CH=CH, JG=JG, KS=KS, MODE=MODE, AG=(A0, A1, A2, A3)),
        out_shape=jax.ShapeDtypeStruct((D, S), A_q.dtype),
        grid=(NB + 1,),
        in_specs=[cur, nxt, nxt, nxt, first, first, first,
                  full((KS, D)), full((1, D)), full((B, 2 * B)), full((2 * B, B)),
                  full((D, F)), full((D, F)), full((D, F))],
        out_specs=pl.BlockSpec((D, TM), lambda s: (0, jnp.maximum(s - 1, 0))),
        scratch_shapes=[
            pltpu.VMEM((P - 1 + 2 * (P + PB) + 11, D, 2 * B), F32),
            pltpu.VMEM((D // 2, TM), jnp.uint32),
            pltpu.VMEM((PB, D // 2, 2 * B), jnp.uint32),
            pltpu.VMEM((D // 2, TM), jnp.uint32),
            pltpu.VMEM((16, TM), F32),
            pltpu.VMEM((F, D), jnp.uint32),
            pltpu.VMEM((D // 2, F), jnp.uint32),
        ],
        compiler_params=pltpu.CompilerParams(vmem_limit_bytes=100 * 2**20, dimension_semantics=("arbitrary",)),
    )(qT, kT, vT, A_ssm_k, kT, vT, A_ssm_k, A_shift_k.T, A_ssm_D.reshape(1, D), ft, fi,
      B_w_gate, B_w_up, B_w_down.T)
    return jnp.swapaxes(oT.reshape(1, D, S), 1, 2)
```

```python
import functools
import numpy as np
import jax
import jax.numpy as jnp
from jax import lax
import jax.experimental.pallas as pl
import jax.experimental.pallas.tpu as pltpu

B = 128
PB = 2
TM = PB * B
GELU_C = 0.7978845608028654
EPS = 1e-5
F32 = jnp.float32
BF16 = jnp.bfloat16


def _dft_tables():
    n = np.arange(B)[:, None]
    k = np.arange(B)[None, :]
    ang = 2.0 * np.pi * (((2 * k + 1) * n) % (4 * B)) / (4 * B)
    ft = np.concatenate([np.cos(ang), -np.sin(ang)], axis=1)
    return ft.astype(np.float32), (ft.T / B).astype(np.float32)


def _stat_terms(x, y, cb):
    a = x - cb
    ay = a * y
    return a, a * a, ay, a * ay, ay * y, ay * ay


def _rsqrt_valu(x):
    i = lax.bitcast_convert_type(x, jnp.int32)
    y = lax.bitcast_convert_type(jnp.int32(0x5F3759DF) - lax.shift_right_logical(i, jnp.int32(1)), F32)
    hx = 0.5 * x
    for _ in range(4):
        y = y * (1.5 - hx * y * y)
    return y


def _stats(c, sums, y1, y2, d, rsqrt=lax.rsqrt):
    s1, s2, t1, t2, v1, v2 = [jnp.sum(t, axis=0, keepdims=True) for t in sums]
    inv = 1.0 / d
    m = s1 * inv
    e2 = s2 * inv
    r = rsqrt(jnp.maximum(e2 - m * m, 0.0) + EPS)
    mb = m + r * (t1 - m * y1) * inv
    eb = e2 + (2.0 * inv) * r * (t2 - m * t1) + (r * r * inv) * (v2 - 2.0 * m * v1 + m * m * y2)
    r3 = rsqrt(jnp.maximum(eb - mb * mb, 0.0) + EPS)
    return c + m, r, c + mb, r3


def _acc(accs, vals):
    return list(vals) if accs is None else [a + v for a, v in zip(accs, vals)]


def _gelu(x):
    inner = x * (GELU_C + (GELU_C * 0.044715) * (x * x))
    return (0.5 * x) * (1.0 + jnp.tanh(inner))


def _pack(x):
    return pltpu.bitcast(x, jnp.uint32)


def _unpack(x):
    return pltpu.bitcast(x, BF16)


_TN = (((0,), (0,)), ((), ()))


def _kernel(q_hbm, k_hbm, v_hbm, h_hbm, sk_hbm, d_hbm, ft_hbm, fi_hbm, wg_hbm, wu_hbm, wdt_hbm,
            o_hbm,
            ob, ug_ref, kv_ref, yf_ref, xn_ref, ys_ref, wt_ref, wd_ref, kp_ref,
            qb, kb, vb, hb, sk_ref, d_ref, ft_ref, fi_ref, wg_ref, wu_ref, wdt_ref,
            sem,
            *, D, F, NB, CH, JG, KS, MODE, AG, HOLD, UR, BG, T0, DT, GRID):
    s = pl.program_id(0)
    P = NB * PB
    PAD = P - 1
    UBASE = PAD
    HBASE = PAD + P + PB
    ZP = HBASE + P + PB
    KVD, YST, CB, FENCE, YY, X1, X2, X3 = ZP + 1, ZP + 2, ZP + 3, ZP + 6, ZP + 7, ZP + 8, ZP + 9, ZP + 10
    zd = jnp.minimum(s, 0)
    lo, hi = slice(0, B), slice(B, 2 * B)
    starts = [sum(CH[:i]) for i in range(len(CH))]
    NC = len(CH)
    Q, K, V, H = 0, 1, 2, 3
    G, U, DW = 0, 1, 2
    streams = ((q_hbm, qb), (k_hbm, kb), (v_hbm, vb), (h_hbm, hb))

    def blk_copy(i, b):
        src_ref, buf = streams[i]
        start = b * TM if isinstance(b, int) else pl.multiple_of(b * TM, TM)
        return pltpu.make_async_copy(src_ref.at[:, pl.ds(start, TM)], buf.at[b], sem.at[4 + 3 * NC + i * NB + b])

    def w_copy(i, c):
        src_ref, buf = ((wg_hbm, wg_ref), (wu_hbm, wu_ref), (wdt_hbm, wdt_ref))[i]
        cs = pl.ds(starts[c], CH[c])
        return pltpu.make_async_copy(src_ref.at[:, cs], buf.at[:, cs], sem.at[4 + i * NC + c])

    def small_copy(i):
        src_ref, buf = ((sk_hbm, sk_ref), (d_hbm, d_ref), (ft_hbm, ft_ref), (fi_hbm, fi_ref))[i]
        return pltpu.make_async_copy(src_ref, buf, sem.at[i])

    def out_copy(b):
        start = b * TM if isinstance(b, int) else pl.multiple_of(b * TM, TM)
        return pltpu.make_async_copy(ob.at[b], o_hbm.at[:, pl.ds(start, TM)], sem.at[4 + 3 * NC + 4 * NB + b])

    def emit(x4, b):
        ob[b] = x4.astype(ob.dtype)
        out_copy(b).start()

    def wait(*cs):
        for c in cs:
            c.wait()

    def init():
        rows = lax.broadcasted_iota(jnp.int32, (16, D), 0)
        a = jnp.zeros((16, D), F32)
        skf = sk_ref[...].astype(F32)
        for j in range(KS):
            a = jnp.where(rows == j, jnp.broadcast_to(skf[j:j + 1, :], (16, D)), a)
        er = lax.broadcasted_iota(jnp.int32, (16, KS * B), 0)
        ec = lax.broadcasted_iota(jnp.int32, (16, KS * B), 1) // B
        e = jnp.where(er == ec, 1.0, 0.0).astype(BF16)
        t = lax.dot_general(a.astype(BF16), e, _TN, preferred_element_type=F32)
        for j in range(KS // 2):
            ug_ref[CB + j] = t[:, 2 * j * B:2 * (j + 1) * B]

    def init_d():
        rows = lax.broadcasted_iota(jnp.int32, (16, D), 0)
        a = jnp.where(rows == 0, jnp.broadcast_to(d_ref[...].astype(F32), (16, D)), 0.0)
        e = jnp.where(lax.broadcasted_iota(jnp.int32, (16, B), 0) == 0, 1.0, 0.0).astype(BF16)
        ug_ref[CB + 2, :, lo] = lax.dot_general(a.astype(BF16), e, _TN, preferred_element_type=F32)

    def kv_rows(r0, nr, parts, kr, vr, z):
        rs = slice(r0, r0 + nr)
        hs = slice(r0 // 2, (r0 + nr) // 2)
        lane = lax.broadcasted_iota(jnp.int32, (nr // 2, B), 1)
        if not isinstance(z, int) and (MODE & 2):
            lane = lane + lax.bitcast_convert_type(ug_ref[z, 0:nr // 2, lo], jnp.int32)
        taps = [ug_ref[CB + z + j // 2, rs, (lo, hi)[j % 2]] for j in range(KS)]
        dcol = ug_ref[CB + 2 + z, rs, lo]
        p = parts[0]
        kp = kp_ref[hs, :] if p == 0 else _pack(kr[rs, (p - 1) * B:p * B])
        for p in parts:
            ps = slice(p * B, (p + 1) * B)
            kcb = kr[rs, ps]
            kc = _pack(kcb)
            acc = kcb.astype(F32) * taps[0]
            for j in range(1, KS):
                sh = pltpu.roll(jnp.where(lane >= B - j, kp, kc), j, 1)
                acc = acc + _unpack(sh).astype(F32) * taps[j]
            kvb = (acc * vr[rs, ps].astype(F32)).astype(BF16)
            kv_ref[hs, ps] = _pack(kvb)
            ug_ref[KVD, rs, ps] = kvb.astype(F32) * dcol
            kp = kc
        if parts[-1] == PB - 1:
            kp_ref[hs, :] = kp

    def fwd_h(hr, blk):
        p0 = jnp.minimum(blk, NB) * PB
        for p in range(PB):
            ug_ref[HBASE + p0 + p] = jnp.dot(hr[:, p * B:(p + 1) * B], ft_ref[...], preferred_element_type=F32)

    def fwd_u(blk):
        p0 = jnp.minimum(blk, NB) * PB
        for p in range(PB):
            ug_ref[UBASE + p0 + p] = jnp.dot(_unpack(kv_ref[:, p * B:(p + 1) * B]), ft_ref[...], preferred_element_type=F32)

    def mac_rows(r, nj, blk, chained):
        p0 = blk * PB
        gmax = p0 + PB - 1
        rs = slice(r * 8, (r + 1) * 8)
        sgn = jnp.where(lax.broadcasted_iota(jnp.int32, (8, B), 1) % 2 == 0, 1.0, -1.0)
        ar = [None] * PB
        ai = [None] * PB
        us = {}
        static = isinstance(blk, int)
        z = (zd if chained else 0)
        for j in range(nj):
            gj = HBASE + (j + z if static else jnp.minimum(j, gmax))
            gr = ug_ref[gj, rs, lo]
            gi = ug_ref[gj, rs, hi]
            for p in range(PB):
                off = p - j
                if static and p0 + off < 0:
                    continue
                if off not in us:
                    ui_ = UBASE + p0 + off + (z if static else 0)
                    us[off] = (ug_ref[ui_, rs, lo], ug_ref[ui_, rs, hi])
                ur, ui = us[off]
                tr = ur * gr - ui * gi
                ti = ur * gi + ui * gr
                ar[p] = tr if ar[p] is None else ar[p] + tr
                ai[p] = ti if ai[p] is None else ai[p] + ti
            if chained and (j + 1) % JG == 0 and j + 1 < nj:
                for p in range(PB):
                    ug_ref[FENCE, p * 8:(p + 1) * 8, lo] = ar[p]
                    ug_ref[FENCE, p * 8:(p + 1) * 8, hi] = ai[p]
        out = []
        if static and blk == 0:
            zr = zi = None
        else:
            zr, zi = ug_ref[ZP + z, rs, lo], ug_ref[ZP + z, rs, hi]
        for p in range(PB):
            out.append((ar[p], ai[p]) if zr is None else (ar[p] - sgn * zi, ai[p] + sgn * zr))
            zr, zi = ar[p], ai[p]
        ug_ref[ZP, rs, lo] = zr
        ug_ref[ZP, rs, hi] = zi
        if chained:
            ug_ref[FENCE, 0:8, lo] = out[0][0]
            ug_ref[FENCE, 0:8, hi] = out[0][1]
        return out

    def mac_group(g, nj, blk, chained=True):
        res = [mac_rows(2 * g + i, nj, blk, chained) for i in range(2)]
        rs = slice(g * 8, (g + 1) * 8)
        for p in range(PB):
            yf_ref[p, rs, lo] = _pack(jnp.concatenate([x[p][0] for x in res], axis=0).astype(BF16))
            yf_ref[p, rs, hi] = _pack(jnp.concatenate([x[p][1] for x in res], axis=0).astype(BF16))

    def inv_dot():
        for p in range(PB):
            ps = slice(p * B, (p + 1) * B)
            ug_ref[YST, :, ps] = jnp.dot(_unpack(yf_ref[p]), fi_ref[...], preferred_element_type=F32) + ug_ref[KVD, :, ps]

    def side_post(z, old, qr, kr, vr, anchors=None, zero_fill=False):
        anchors = anchors or {}
        NU = D // UR
        c = qr[0:16, :].astype(F32)[0:1]
        cb = jnp.broadcast_to(c, (8, TM))
        accs = None
        for g in range(D // UR):
            rs = slice(g * UR, (g + 1) * UR)
            if g in anchors:
                ug_ref[FENCE, 8:16, lo] = anchors[g]
            if old is not None:
                x = ug_ref[X2 + z, rs, :]
                ug_ref[X3, rs, :] = x + (x - old[0]) * old[1] * ug_ref[YY + z, rs, :]
            x = qr[rs, :].astype(F32)
            y = ug_ref[YST + z, rs, :]
            for i in range(UR // 8):
                yi = y[i * 8:(i + 1) * 8]
                accs = _acc(accs, _stat_terms(x[i * 8:(i + 1) * 8], yi, cb) + (yi, yi * yi))
            if kr is not None:
                kv_rows(g * UR, UR, (0,), kr, vr, z)
            if zero_fill:
                for i in range(0, PAD // 2):
                    ug_ref[i + z, rs, :] = jnp.zeros((UR, 2 * B), F32)
        y1 = jnp.sum(accs[6], axis=0, keepdims=True)
        y2 = jnp.sum(accs[7], axis=0, keepdims=True)
        ys_ref[0:1, :] = y1
        ys_ref[8:9, :] = y2
        mu, r, mu3, r3 = _stats(c, accs[:6], y1, y2, D, _rsqrt_valu if kr is not None else lax.rsqrt)
        for g in range(D // UR):
            rs = slice(g * UR, (g + 1) * UR)
            if NU + g in anchors:
                ug_ref[FENCE, 8:16, lo] = anchors[NU + g]
            x = qr[rs, :].astype(F32)
            y = ug_ref[YST + z, rs, :]
            xo = x + (x - mu) * r * y
            xn = (xo - mu3) * r3
            xn_ref[g * UR // 2:(g + 1) * UR // 2, :] = _pack(xn.astype(BF16))
            ug_ref[YY, rs, :] = y
            ug_ref[X1, rs, :] = xo
            if kr is not None:
                ug_ref[FENCE, 0:8, lo] = xn[UR - 8:UR, B:2 * B]
                kv_rows(g * UR, UR, (1,), kr, vr, z)
            if zero_fill:
                for i in range(PAD // 2, PAD):
                    ug_ref[i + z, rs, :] = jnp.zeros((UR, 2 * B), F32)

    def gu_rows(f0, fc, xn):
        return jnp.dot(_unpack(wt_ref[f0:f0 + fc, :]), xn, preferred_element_type=F32)

    def gu(c, xn):
        return gu_rows(starts[c], CH[c], xn)

    def gu_first(c, n_now, xn):
        f0, fc = starts[c], CH[c]
        pieces = []
        for f in range(f0, f0 + fc, B):
            gt = wg_ref[:, f:f + B].T
            ut = wu_ref[:, f:f + B].T
            pieces += [t[16 * i:16 * (i + 1)] for i in range(B // 16) for t in (gt, ut)]
        lhs = jnp.concatenate(pieces, axis=0)
        wt_ref[f0:f0 + fc, :] = _pack(lhs)
        return jnp.dot(lhs[0:2 * n_now], xn, preferred_element_type=F32)

    def act(r):
        hs = [(_gelu(r[32 * i:32 * i + 16]) * r[32 * i + 16:32 * i + 32]).astype(BF16) for i in range(r.shape[0] // 32)]
        return jnp.concatenate(hs, axis=0)

    def dn(c, hh, acc):
        f0, fc = starts[c], CH[c]
        return jnp.dot(_unpack(wd_ref[:, f0:f0 + fc]), hh, preferred_element_type=F32) + acc

    def dn_first(c, hh, acc):
        f0, fc = starts[c], CH[c]
        w = wdt_ref[:, f0:f0 + fc]
        wd_ref[:, f0:f0 + fc] = _pack(w)
        return jnp.dot(w, hh, preferred_element_type=F32) + acc

    def mlp(xn, side, first_acc, res_slot):
        raws = [gu(0, xn), gu(1, xn)]
        accs = []
        acc = None
        for c in range(NC - 1):
            if c >= 1:
                raws.append(gu(c + 1, xn))
            acc = dn(c, act(raws[c]), first_acc() if c == 0 else acc)
            accs.append(acc)
        side(raws, accs)
        if res_slot is not None:
            acc = acc + ug_ref[res_slot]
        return dn(NC - 1, act(raws[NC - 1]), acc)

    def tail(v, t):
        n = v.shape[0]
        return v[n - 8:n, (lo, hi)[t]]

    def paced(seq, n_units, t0, dt):
        anchors = {}
        for u in range(n_units):
            t = t0 + dt * u
            for val in seq:
                n = val.shape[0]
                if t < 2 * n:
                    r = (t % n) // 8 * 8
                    anchors[u] = val[r:r + 8, (lo, hi)[t // n]]
                    break
                t -= 2 * n
        return anchors

    def mid_norm(x2):
        ug_ref[X2] = x2
        st = []
        for p in range(PB):
            ps = slice(p * B, (p + 1) * B)
            c = x2[0:1, ps]
            cb = jnp.broadcast_to(c, (8, B))
            accs = None
            for i in range(D // 8):
                accs = _acc(accs, _stat_terms(x2[i * 8:(i + 1) * 8, ps], ug_ref[YY, i * 8:(i + 1) * 8, ps], cb))
            st.append(_stats(c, accs, ys_ref[0:1, ps], ys_ref[8:9, ps], D))
        xn3 = []
        for p in range(PB):
            ps = slice(p * B, (p + 1) * B)
            mu, r, mu3, r3 = st[p]
            x2r = ug_ref[X2 + (zd if p > 0 else 0), :, ps]
            xn3.append(((x2r + (x2r - mu) * r * ug_ref[YY, :, ps] - mu3) * r3).astype(BF16))
        old = [jnp.concatenate([st[p][i] for p in range(PB)], axis=1) for i in range(2)]
        return jnp.concatenate(xn3, axis=1), old

    def second_half(x2, qr, kr, vr, hr, blk):
        inv_dot()
        xn3, old = mid_norm(x2)

        def side2(raws, accs):
            seq = [raws[0], raws[1], accs[0], raws[2], accs[1], raws[3]]
            side_post(zd, old, qr, kr, vr, paced(seq, 2 * D // UR, T0, DT))

        x4 = mlp(xn3, side2, lambda: jnp.zeros((D, TM), F32), X3)
        emit(x4, s)
        fwd_h(hr, blk)
        fwd_u(blk)

    @pl.when(s == 0)
    def _():
        HB = HOLD
        order = [small_copy(i) for i in range(4)]
        order += [blk_copy(i, 0) for i in (K, V, H, Q)]
        order += [w_copy(i, c) for c in range(3) for i in (G, U)]
        order += [w_copy(DW, 0), w_copy(G, 3), w_copy(U, 3), w_copy(DW, 1), w_copy(DW, 2), w_copy(DW, 3)]
        order += [blk_copy(i, 1) for i in (K, V, H, Q)] + [blk_copy(i, 2) for i in (K, V, H)]
        late = [blk_copy(Q, 2)] + [blk_copy(i, b_) for b_ in range(3, NB) for i in (K, V, H, Q)]
        for c in order:
            c.start()
        kp_ref[...] = jnp.zeros(kp_ref.shape, jnp.uint32)
        wait(small_copy(0), small_copy(1), small_copy(2), small_copy(3))
        init()
        wait(blk_copy(K, 0), blk_copy(V, 0))
        for c in late:
            c.start()
        init_d()
        kv_rows(0, D, (0, 1), kb.at[0], vb.at[0], 0)
        fwd_u(0)
        wait(blk_copy(H, 0), blk_copy(Q, 0))
        fwd_h(hb.at[0], 0)
        for g in range(D // 16):
            mac_group(g, PB, 0, chained=False)
        inv_dot()
        side_post(0, None, qb.at[0], None, None)

        wait(w_copy(G, 0), w_copy(U, 0))
        xn = _unpack(xn_ref[...])
        h0a = act(gu_first(0, CH[0] - HB, xn))

        wait(w_copy(G, 1), w_copy(U, 1))
        h0b = act(gu_rows(starts[1] - HB, HB, xn))
        h1a = act(gu_first(1, CH[1] - HB, xn))

        wait(w_copy(G, 2), w_copy(U, 2))
        h1b = act(gu_rows(starts[2] - HB, HB, xn))
        h2a = act(gu_first(2, CH[2] - HB, xn))

        wait(w_copy(DW, 0), w_copy(G, 3), w_copy(DW, 1), w_copy(U, 3))
        h2b = act(gu_rows(starts[3] - HB, HB, xn))
        acc = dn_first(0, jnp.concatenate([h0a, h0b], axis=0), ug_ref[X1])
        h3 = act(gu_first(3, CH[3], xn))
        acc = dn_first(1, jnp.concatenate([h1a, h1b], axis=0), acc)

        wait(w_copy(DW, 2), w_copy(DW, 3), blk_copy(K, 1), blk_copy(V, 1), blk_copy(H, 1))
        acc2 = dn_first(2, jnp.concatenate([h2a, h2b], axis=0), acc)
        anchors = paced([acc2], D // 16, 0, 30)
        for g in range(D // 16):
            ug_ref[FENCE, 0:8, lo] = anchors[g]
            kv_rows(g * 16, 16, (0, 1), kb.at[1], vb.at[1], zd)
        x2 = dn_first(3, h3, acc2)
        fwd_h(hb.at[1], 1)
        fwd_u(1)
        xn3, old = mid_norm(x2)
        r0 = gu(0, xn3)
        anchors = paced([r0], D // 16, 0, 64)
        for g in range(D // 16):
            ug_ref[FENCE, 0:8, lo] = anchors[g]
            mac_group(g, 2 * PB, 1)
        hh0 = act(r0)

        wait(blk_copy(Q, 1), blk_copy(K, 2), blk_copy(V, 2), blk_copy(H, 2))
        inv_dot()
        r1 = gu(1, xn3)
        a0 = dn(0, hh0, jnp.zeros((D, TM), F32))
        r2 = gu(2, xn3)
        a1 = dn(1, act(r1), a0)
        r3 = gu(3, xn3)
        a2 = dn(2, act(r2), a1)
        side_post(zd, old, qb.at[1], kb.at[2], vb.at[2], paced([r1, a0, r2, a1, r3], 2 * D // UR, 64, DT), True)
        x4 = dn(3, act(r3), a2 + ug_ref[X3])
        emit(x4, 0)
        fwd_h(hb.at[2], 2)
        fwd_u(2)
        wait(*late)
        if GRID == 1:
            wait(out_copy(0))

    @pl.when(s > 0)
    def _():
        def side1(raws, accs):
            anchors = {0: raws[0][0:8, lo], AG[0]: tail(raws[0], 0), AG[1]: tail(raws[0], 1),
                       AG[2]: tail(raws[1], 0), AG[3]: tail(raws[1], 1)}
            for g in range(D // 16):
                if g in anchors:
                    ug_ref[FENCE, 0:8, lo] = anchors[g]
                mac_group(g, P, s + 1)

        x2 = mlp(_unpack(xn_ref[...]), side1, lambda: ug_ref[X1], None)
        n1 = jnp.minimum(s + 1, NB - 1)
        n2 = jnp.minimum(s + 2, NB - 1)
        second_half(x2, qb.at[n1], kb.at[n2], vb.at[n2], hb.at[n2], s + 2)

    @pl.when(s == NB - 1)
    def _():
        wait(*[out_copy(b_) for b_ in range(NB)])


@jax.jit
def pallas_interleave_layers__ssm_conv_h3__geglu_ffn__prompt_kernel(
        A_q, A_k, A_v, A_shift_k, A_ssm_k, A_ssm_D, B_x, B_w_gate, B_w_up, B_w_down):
    CHK = 0
    JG = 4
    MODE = 0
    A0 = 6
    A1 = 10
    A2 = 14
    A3 = 99
    HOLD = 128
    UR = 16
    BGK = 0
    T0 = 1200
    DT = 110
    GRID = 0
    BGS = {0: (5, 10, 16, 19, 21, 27, 99), 1: (4, 9, 15, 18, 20, 26, 99), 2: (6, 12, 18, 20, 23, 99, 99), 3: (99,) * 7, 4: (10, 26, 42, 50, 99, 99, 99), 5: (8, 22, 36, 44, 52, 99, 99)}
    CH = {0: (512, 512, 512, 256)}[CHK]
    _, S, D = A_q.shape
    F = B_w_gate.shape[1]
    KS = A_shift_k.shape[1]
    NB = S // TM
    P = S // B
    ft, fi = _dft_tables()
    ft = jnp.asarray(ft, BF16)
    fi = jnp.asarray(fi, BF16)
    qT = jnp.swapaxes(A_q, 1, 2).reshape(D, S)
    kT = jnp.swapaxes(A_k, 1, 2).reshape(D, S)
    vT = jnp.swapaxes(A_v, 1, 2).reshape(D, S)
    hbm = pl.BlockSpec(memory_space=pl.ANY)
    oT = pl.pallas_call(
        functools.partial(_kernel, D=D, F=F, NB=NB, CH=CH, JG=JG, KS=KS, MODE=MODE, AG=(A0, A1, A2, A3), HOLD=HOLD, UR=UR, BG=BGS[BGK], T0=T0, DT=DT, GRID=GRID),
        out_shape=jax.ShapeDtypeStruct((D, S), A_q.dtype),
        grid=(GRID or NB,),
        in_specs=[hbm] * 11,
        out_specs=hbm,
        scratch_shapes=[
            pltpu.VMEM((NB, D, TM), BF16),
            pltpu.VMEM((P - 1 + 2 * (P + PB) + 11, D, 2 * B), F32),
            pltpu.VMEM((D // 2, TM), jnp.uint32),
            pltpu.VMEM((PB, D // 2, 2 * B), jnp.uint32),
            pltpu.VMEM((D // 2, TM), jnp.uint32),
            pltpu.VMEM((16, TM), F32),
            pltpu.VMEM((F, D), jnp.uint32),
            pltpu.VMEM((D // 2, F), jnp.uint32),
            pltpu.VMEM((D // 2, B), jnp.uint32),
            pltpu.VMEM((NB, D, TM), BF16),
            pltpu.VMEM((NB, D, TM), BF16),
            pltpu.VMEM((NB, D, TM), BF16),
            pltpu.VMEM((NB, D, TM), BF16),
            pltpu.VMEM((KS, D), BF16),
            pltpu.VMEM((1, D), BF16),
            pltpu.VMEM((B, 2 * B), BF16),
            pltpu.VMEM((2 * B, B), BF16),
            pltpu.VMEM((D, F), BF16),
            pltpu.VMEM((D, F), BF16),
            pltpu.VMEM((D, F), BF16),
            pltpu.SemaphoreType.DMA((4 + 3 * len(CH) + 5 * NB,)),
        ],
        compiler_params=pltpu.CompilerParams(vmem_limit_bytes=100 * 2**20, dimension_semantics=("arbitrary",)),
    )(qT, kT, vT, A_ssm_k, A_shift_k.T, A_ssm_D.reshape(1, D), ft, fi,
      B_w_gate, B_w_up, B_w_down.T)
    return jnp.swapaxes(oT.reshape(1, D, S), 1, 2)
```

```python
import functools

import numpy as np
import jax
import jax.numpy as jnp
from jax import lax
import jax.experimental.pallas as pl
import jax.experimental.pallas.tpu as pltpu

B = 128
PB = 2
TM = PB * B
UR = 16
GELU_C = 0.7978845608028654
EPS = 1e-5
F32 = jnp.float32
BF16 = jnp.bfloat16
U32 = jnp.uint32
_TN = (((0,), (0,)), ((), ()))


def _dft_tables():
    n = np.arange(B)[:, None]
    k = np.arange(B)[None, :]
    ang = 2.0 * np.pi * (((2 * k + 1) * n) % (4 * B)) / (4 * B)
    ft = np.concatenate([np.cos(ang), -np.sin(ang)], axis=1)
    return ft.astype(np.float32), (ft.T / B).astype(np.float32)


def _gelu(x):
    inner = x * (GELU_C + (GELU_C * 0.044715) * (x * x))
    return (0.5 * x) * (1.0 + jnp.tanh(inner))


def _pack(x):
    return pltpu.bitcast(x, U32)


def _unpack(x):
    return pltpu.bitcast(x, BF16)


def _rsqrt_valu(x):
    i = lax.bitcast_convert_type(x, jnp.int32)
    y = lax.bitcast_convert_type(jnp.int32(0x5F3759DF) - lax.shift_right_logical(i, jnp.int32(1)), F32)
    hx = 0.5 * x
    for _ in range(4):
        y = y * (1.5 - hx * y * y)
    return y


def _stat_terms(x, y, pivot):
    a = x - pivot
    ay = a * y
    return a, a * a, ay, a * ay, ay * y, ay * ay


def _acc(accs, vals):
    return list(vals) if accs is None else [a + v for a, v in zip(accs, vals)]


def _stats(pivot, sums, y1, y2, ys, d, rsqrt):
    s1, s2, t1, t2, v1, v2 = [jnp.sum(t, axis=0, keepdims=True) for t in sums]
    inv = 1.0 / d
    m = s1 * inv
    e2 = s2 * inv
    r = rsqrt(jnp.maximum(e2 - m * m, 0.0) + EPS)
    mb = m + (r * (t1 - m * y1) * inv) * ys
    quad = (r * r * inv) * (v2 - 2.0 * m * v1 + m * m * y2)
    eb = e2 + ((2.0 * inv) * r * (t2 - m * t1)) * ys + (quad * ys) * ys
    r3 = rsqrt(jnp.maximum(eb - mb * mb, 0.0) + EPS)
    return pivot + m, r * ys, pivot + mb, r3


def _kernel(q_hbm, k_hbm, v_hbm, h_hbm, sk_hbm, d_hbm, ft_hbm, fi_hbm, wg_hbm, wu_hbm, wdt_hbm,
            o_hbm,
            ob, ug_ref, kv_ref, yf_ref, xn_ref, ys_ref, wt_ref, wd_ref, kp_ref, hh_ref,
            qb, kb, vb, hb, sk_ref, d_ref, ft_ref, fi_ref, wg_ref, wu_ref, wdt_ref,
            sem,
            *, D, F, NB, KS, CH, cfg):
    s = pl.program_id(0)
    P = NB * PB
    PAD = P - 1
    NC = len(CH)
    NU = D // UR
    NZ = cfg["NZ"]
    starts = [sum(CH[:i]) for i in range(NC)]
    lo, hi = slice(0, B), slice(B, 2 * B)

    UBASE = PAD
    HBASE = PAD + P + PB
    ZP = HBASE + P + PB
    KVD, CB, FENCE, YY, X1, X2, X3, YST = (ZP + i for i in (1, 2, 5, 6, 7, 8, 9, 10))

    zd = jnp.minimum(s, 0)

    Q, K, V, H = range(4)
    G, U, DW = range(3)

    def small_copy(i):
        src, dst = ((sk_hbm, sk_ref), (d_hbm, d_ref), (ft_hbm, ft_ref), (fi_hbm, fi_ref))[i]
        return pltpu.make_async_copy(src, dst, sem.at[i])

    def w_copy(i, c):
        src, dst = ((wg_hbm, wg_ref), (wu_hbm, wu_ref), (wdt_hbm, wdt_ref))[i]
        cs = pl.ds(starts[c], CH[c])
        return pltpu.make_async_copy(src.at[:, cs], dst.at[:, cs], sem.at[4 + i * NC + c])

    def blk_copy(i, b):
        src, dst = ((q_hbm, qb), (k_hbm, kb), (v_hbm, vb), (h_hbm, hb))[i]
        return pltpu.make_async_copy(src.at[:, pl.ds(b * TM, TM)], dst.at[b], sem.at[4 + 3 * NC + i * NB + b])

    def out_copy(b):
        start = b * TM if isinstance(b, int) else pl.multiple_of(b * TM, TM)
        return pltpu.make_async_copy(ob.at[b], o_hbm.at[:, pl.ds(start, TM)], sem.at[4 + 3 * NC + 4 * NB + b])

    def wait(*copies):
        for c in copies:
            c.wait()

    def init_taps():
        rows = lax.broadcasted_iota(jnp.int32, (16, D), 0)
        a = jnp.zeros((16, D), F32)
        skf = sk_ref[...].astype(F32)
        for j in range(KS):
            a = jnp.where(rows == j, jnp.broadcast_to(skf[j:j + 1, :], (16, D)), a)
        er = lax.broadcasted_iota(jnp.int32, (16, KS * B), 0)
        ec = lax.broadcasted_iota(jnp.int32, (16, KS * B), 1) // B
        e = jnp.where(er == ec, 1.0, 0.0).astype(BF16)
        t = lax.dot_general(a.astype(BF16), e, _TN, preferred_element_type=F32)
        for j in range(KS // 2):
            ug_ref[CB + j] = t[:, 2 * j * B:2 * (j + 1) * B]

    def init_d():
        rows = lax.broadcasted_iota(jnp.int32, (16, D), 0)
        a = jnp.where(rows == 0, jnp.broadcast_to(d_ref[...].astype(F32).reshape(1, D), (16, D)), 0.0)
        e = jnp.where(lax.broadcasted_iota(jnp.int32, (16, B), 0) == 0, 1.0, 0.0).astype(BF16)
        ug_ref[CB + 2, :, lo] = lax.dot_general(a.astype(BF16), e, _TN, preferred_element_type=F32)

    def kv_rows(r0, nr, parts, kr, vr, z):
        rs = slice(r0, r0 + nr)
        hs = slice(r0 // 2, (r0 + nr) // 2)
        lane = lax.broadcasted_iota(jnp.int32, (nr // 2, B), 1)
        taps = [ug_ref[CB + z + j // 2, rs, (lo, hi)[j % 2]] for j in range(KS)]
        dcol = ug_ref[CB + 2 + z, rs, lo]
        p = parts[0]
        kp = kp_ref[hs, :] if p == 0 else _pack(kr[rs, (p - 1) * B:p * B])
        for p in parts:
            ps = slice(p * B, (p + 1) * B)
            kcb = kr[rs, ps]
            kc = _pack(kcb)
            acc = kcb.astype(F32) * taps[0]
            for j in range(1, KS):
                sh = pltpu.roll(jnp.where(lane >= B - j, kp, kc), j, 1)
                acc = acc + _unpack(sh).astype(F32) * taps[j]
            kv_ref[hs, ps] = _pack((acc * vr[rs, ps].astype(F32)).astype(BF16))
            ug_ref[KVD, rs, ps] = _unpack(kv_ref[hs, ps]).astype(F32) * dcol
            kp = kc
        if parts[-1] == PB - 1:
            kp_ref[hs, :] = kp

    def fwd_h(hr, blk):
        for p in range(PB):
            ug_ref[HBASE + blk * PB + p] = jnp.dot(hr[:, p * B:(p + 1) * B], ft_ref[...],
                                                   preferred_element_type=F32)

    def fwd_u(blk):
        for p in range(PB):
            ug_ref[UBASE + blk * PB + p] = jnp.dot(_unpack(kv_ref[:, p * B:(p + 1) * B]), ft_ref[...],
                                                   preferred_element_type=F32)

    def mac_rows(r, nj, blk, chained):
        p0 = blk * PB
        rs = slice(r * 8, (r + 1) * 8)
        sgn = jnp.where(lax.broadcasted_iota(jnp.int32, (8, B), 1) % 2 == 0, 1.0, -1.0)
        static = isinstance(blk, int)
        z = zd if chained else 0
        ar = [None] * PB
        ai = [None] * PB
        us = {}
        for j in range(nj):
            gj = HBASE + (j + z if static else jnp.minimum(j, p0 + PB - 1))
            gr = ug_ref[gj, rs, lo]
            gi = ug_ref[gj, rs, hi]
            for p in range(PB):
                off = p - j
                if static and p0 + off < 0:
                    continue
                if off not in us:
                    ix = UBASE + p0 + off + (z if static else 0)
                    us[off] = (ug_ref[ix, rs, lo], ug_ref[ix, rs, hi])
                ur, ui = us[off]
                tr = ur * gr - ui * gi
                ti = ur * gi + ui * gr
                ar[p] = tr if ar[p] is None else ar[p] + tr
                ai[p] = ti if ai[p] is None else ai[p] + ti
            if chained and (j + 1) % cfg["JG"] == 0 and j + 1 < nj:
                for p in range(PB):
                    ug_ref[FENCE, p * 8:(p + 1) * 8, lo] = ar[p]
                    ug_ref[FENCE, p * 8:(p + 1) * 8, hi] = ai[p]
        zr = zi = None
        if not (static and blk == 0):
            zr, zi = ug_ref[ZP + z, rs, lo], ug_ref[ZP + z, rs, hi]
        out = []
        for p in range(PB):
            out.append((ar[p], ai[p]) if zr is None else (ar[p] - sgn * zi, ai[p] + sgn * zr))
            zr, zi = ar[p], ai[p]
        ug_ref[ZP, rs, lo] = zr
        ug_ref[ZP, rs, hi] = zi
        if chained:
            ug_ref[FENCE, 0:8, lo] = out[0][0]
            ug_ref[FENCE, 0:8, hi] = out[0][1]
        return out

    def mac(nj, blk, anchors):
        for g in range(NU):
            if anchors and g in anchors:
                ug_ref[FENCE, 0:8, lo] = anchors[g]
            res = [mac_rows(2 * g + i, nj, blk, anchors is not None) for i in range(2)]
            for p in range(PB):
                for i in range(2):
                    yf_ref[g * 8:(g + 1) * 8, (2 * p + i) * B:(2 * p + i + 1) * B] = _pack(
                        jnp.concatenate([x[p][i] for x in res], axis=0).astype(BF16))

    def inv_dot():
        for p in range(PB):
            for i in range(2):
                ug_ref[YST + i, :, p * B:(p + 1) * B] = jnp.dot(
                    _unpack(yf_ref[:, (2 * p + i) * B:(2 * p + i + 1) * B]), fi_ref[i * B:(i + 1) * B, :],
                    preferred_element_type=F32)

    def side_post(old, qr, kr, vr, anchors, zero_fill=False):
        chained = anchors is not None
        z = zd if chained else 0
        pivot = qr[0:16, :].astype(F32)[0:1]
        pb = jnp.broadcast_to(pivot, (8, TM))
        accs = None
        for g in range(NU):
            rs = slice(g * UR, (g + 1) * UR)
            if chained:
                ug_ref[FENCE, 8:16, lo] = anchors[g]
                x = ug_ref[X2 + z, rs, :]
                ug_ref[X3, rs, :] = x + (x - old[0]) * old[1] * ug_ref[YY + z, rs, :]
            x = qr[rs, :].astype(F32)
            y = ug_ref[YST + z, rs, :] + ug_ref[YST + 1 + z, rs, :] + ug_ref[KVD + z, rs, :]
            ug_ref[YY, rs, :] = y
            for i in range(UR // 8):
                yi = y[i * 8:(i + 1) * 8]
                accs = _acc(accs, _stat_terms(x[i * 8:(i + 1) * 8], yi, pb) + (yi, yi * yi))
            if chained:
                kv_rows(g * UR, UR, (0,), kr, vr, z)
            if zero_fill:
                for i in range(NZ, (NZ + PAD) // 2):
                    ug_ref[i + z, rs, :] = jnp.zeros((UR, 2 * B), F32)
        rsqrt = _rsqrt_valu if chained else lax.rsqrt
        y1 = jnp.sum(accs[6], axis=0, keepdims=True)
        y2 = jnp.sum(accs[7], axis=0, keepdims=True)
        ms = y2 * (1.0 / D) + 1e-30
        sy = rsqrt(ms)
        ys_ref[0:1, :] = y1 * sy
        ys_ref[8:9, :] = (y2 * sy) * sy
        ys_ref[16:17, :] = ms * sy
        mu, r, mu3, r3 = _stats(pivot, accs[:6], y1, y2, 1.0, D, rsqrt)
        for g in range(NU):
            rs = slice(g * UR, (g + 1) * UR)
            if chained:
                ug_ref[FENCE, 8:16, lo] = anchors[NU + g]
            x = qr[rs, :].astype(F32)
            y = ug_ref[YY + z, rs, :]
            xo = x + (x - mu) * r * y
            xn = (xo - mu3) * r3
            xn_ref[g * UR // 2:(g + 1) * UR // 2, :] = _pack(xn.astype(BF16))
            ug_ref[YY, rs, :] = y * sy
            ug_ref[X1, rs, :] = xo
            if chained:
                ug_ref[FENCE, 0:8, lo] = xn[UR - 8:UR, hi]
                kv_rows(g * UR, UR, (1,), kr, vr, z)
            if zero_fill:
                for i in range((NZ + PAD) // 2, PAD):
                    ug_ref[i + z, rs, :] = jnp.zeros((UR, 2 * B), F32)

    def gu_rows(f0, fc, xn):
        return jnp.dot(_unpack(wt_ref[f0:f0 + fc, :]), xn, preferred_element_type=F32)

    def gu(c, xn):
        return gu_rows(starts[c], CH[c], xn)

    def gu_first(c, n_now, xn):
        f0, fc = starts[c], CH[c]
        pieces = []
        for f in range(f0, f0 + fc, B):
            gt = wg_ref[:, f:f + B].T
            ut = wu_ref[:, f:f + B].T
            pieces += [t[16 * i:16 * (i + 1)] for i in range(B // 16) for t in (gt, ut)]
        lhs = jnp.concatenate(pieces, axis=0)
        wt_ref[f0:f0 + fc, :] = _pack(lhs)
        return jnp.dot(lhs[0:2 * n_now], xn, preferred_element_type=F32)

    def act(r, f0):
        for i in range(r.shape[0] // 32):
            h16 = (_gelu(r[32 * i:32 * i + 16]) * r[32 * i + 16:32 * i + 32]).astype(BF16)
            hh_ref[f0 // 2 + 8 * i:f0 // 2 + 8 * (i + 1), :] = _pack(h16)

    def dn(c, acc, first=False):
        f0, fc = starts[c], CH[c]
        if first:
            w = wdt_ref[:, f0:f0 + fc]
            wd_ref[:, f0:f0 + fc] = _pack(w)
        else:
            w = _unpack(wd_ref[:, f0:f0 + fc])
        return jnp.dot(w, _unpack(hh_ref[f0 // 2:(f0 + fc) // 2, :]), preferred_element_type=F32) + acc

    def mlp(xn, acc, side, res_slot, r0=None):
        raws = [gu(0, xn) if r0 is None else r0, gu(1, xn)]
        seq = raws[(r0 is not None):]
        for c in range(NC - 1):
            if c >= 1:
                raws.append(gu(c + 1, xn))
                seq.append(raws[-1])
            if c > 0 or r0 is None:
                act(raws[c], starts[c])
            acc = dn(c, acc)
            seq.append(acc)
        side(seq)
        if res_slot is not None:
            acc = acc + ug_ref[res_slot]
        act(raws[NC - 1], starts[NC - 1])
        return dn(NC - 1, acc)

    def paced(seq, n_units, t0, dt, t1=None, dt1=None):
        anchors = {}
        for u in range(n_units):
            t = t0 + dt * u
            if t1 is not None and u >= n_units // 2:
                t = t1 + dt1 * (u - n_units // 2)
            for val in seq:
                n = val.shape[0]
                if t < PB * n:
                    r = (t % n) // 8 * 8
                    anchors[u] = val[r:r + 8, (lo, hi)[t // n]]
                    break
                t -= PB * n
        return anchors

    def mid_norm(x2):
        ug_ref[X2] = x2
        st = []
        for p in range(PB):
            ps = slice(p * B, (p + 1) * B)
            pivot = x2[0:1, ps]
            pb = jnp.broadcast_to(pivot, (8, B))
            accs = None
            for i in range(D // 8):
                rs = slice(i * 8, (i + 1) * 8)
                accs = _acc(accs, _stat_terms(x2[rs, ps], ug_ref[YY, rs, ps], pb))
            st.append(_stats(pivot, accs, ys_ref[0:1, ps], ys_ref[8:9, ps], ys_ref[16:17, ps], D, lax.rsqrt))
        mu, r, mu3, r3 = [jnp.concatenate([st[p][i] for p in range(PB)], axis=1) for i in range(4)]
        dr = D - cfg["DR"]
        x2h = jnp.concatenate([ug_ref[X2, 0:dr, hi], ug_ref[X2 + zd, dr:D, hi]], axis=0)
        x2r = jnp.concatenate([ug_ref[X2, :, lo], x2h], axis=1)
        xn3 = ((x2r + (x2r - mu) * r * ug_ref[YY] - mu3) * r3).astype(BF16)
        return xn3, (mu, r)

    def emit(x4, b):
        ob[b] = x4.astype(ob.dtype)
        out_copy(b).start()

    zeros = lambda: jnp.zeros((D, TM), F32)

    @pl.when(s == 0)
    def _():
        hb_ = cfg["HOLD"]
        order = [small_copy(0), blk_copy(K, 0), blk_copy(V, 0), small_copy(1), small_copy(2), small_copy(3),
                 blk_copy(H, 0), blk_copy(Q, 0)]
        order += [w_copy(i, c) for c in range(3) for i in (G, U)]
        order += [w_copy(DW, 0), w_copy(G, 3), w_copy(U, 3), w_copy(DW, 1), w_copy(DW, 2), w_copy(DW, 3)]
        order += [blk_copy(i, 1) for i in (K, V, H, Q)] + [blk_copy(i, 2) for i in (K, V)]
        late = [blk_copy(H, 2), blk_copy(Q, 2)] + [blk_copy(i, b) for b in range(3, NB) for i in (K, V, H, Q)]
        for c in order:
            c.start()
        kp_ref[...] = jnp.zeros(kp_ref.shape, U32)
        ug_ref[0:NZ] = jnp.zeros((NZ, D, 2 * B), F32)

        wait(small_copy(0))
        init_taps()

        wait(blk_copy(K, 0), blk_copy(V, 0), small_copy(1), small_copy(2))
        init_d()
        kv_rows(0, D, (0, 1), kb.at[0], vb.at[0], 0)
        fwd_u(0)

        wait(small_copy(3), blk_copy(H, 0), blk_copy(Q, 0))
        fwd_h(hb.at[0], 0)
        mac(PB, 0, None)
        inv_dot()
        side_post(None, qb.at[0], None, None, None)

        wait(w_copy(G, 0), w_copy(U, 0))
        xn = _unpack(xn_ref[...])
        act(gu_first(0, CH[0] - hb_, xn), starts[0])

        wait(w_copy(G, 1), w_copy(U, 1))
        for c in late:
            c.start()
        act(gu_rows(starts[1] - hb_, hb_, xn), starts[1] - hb_)
        act(gu_first(1, CH[1] - hb_, xn), starts[1])

        wait(w_copy(G, 2), w_copy(U, 2))
        act(gu_rows(starts[2] - hb_, hb_, xn), starts[2] - hb_)
        act(gu_first(2, CH[2] - hb_, xn), starts[2])

        wait(w_copy(DW, 0), w_copy(G, 3), w_copy(U, 3), w_copy(DW, 1))
        act(gu_rows(starts[3] - hb_, hb_, xn), starts[3] - hb_)
        acc = dn(0, ug_ref[X1], True)
        act(gu_first(3, CH[3], xn), starts[3])
        acc = dn(1, acc, True)

        wait(w_copy(DW, 2), w_copy(DW, 3), blk_copy(K, 1), blk_copy(V, 1), blk_copy(H, 1))
        acc = dn(2, acc, True)
        anchors = paced([acc], NU, 0, 30)
        for g in range(NU):
            ug_ref[FENCE, 0:8, lo] = anchors[g]
            kv_rows(g * UR, UR, (0, 1), kb.at[1], vb.at[1], zd)
        x2 = dn(3, acc, True)
        fwd_h(hb.at[1], 1)
        fwd_u(1)
        xn3, old = mid_norm(x2)
        r0 = gu(0, xn3)
        mac(2 * PB, 1, paced([r0], NU, 0, 64))
        act(r0, starts[0])

        wait(blk_copy(Q, 1), blk_copy(K, 2), blk_copy(V, 2))
        inv_dot()
        side = lambda seq: side_post(old, qb.at[1], kb.at[2], vb.at[2], paced(seq, 2 * NU, *cfg["FP"]), True)
        emit(mlp(xn3, zeros(), side, X3, r0), 0)
        wait(*late)

    @pl.when(s > 0)
    def _():
        n1 = jnp.minimum(s + 1, NB - 1)
        n2 = jnp.minimum(s + 2, NB - 1)
        fwd_h(hb.at[n1], s + 1)
        fwd_u(s + 1)

        def side1(seq):
            ends = [v[v.shape[0] - 8:, t] for v in seq[:2] for t in (lo, hi)]
            anchors = {0: seq[0][0:8, lo]}
            anchors.update(zip(cfg["AG"], ends))
            mac(P, s + 1, anchors)

        x2 = mlp(_unpack(xn_ref[...]), ug_ref[X1], side1, None)
        inv_dot()
        xn3, old = mid_norm(x2)
        side2 = lambda seq: side_post(old, qb.at[n1], kb.at[n2], vb.at[n2], paced(seq, 2 * NU, *cfg["SP"]))
        emit(mlp(xn3, zeros(), side2, X3), s)

    @pl.when(s == NB - 1)
    def _():
        wait(*[out_copy(b) for b in range(NB)])


_CFG = dict(JG=4, AG=(6, 10, 14), HOLD=128, DR=128,
            SP=(1000, 64, 5700, 72), FP=(64, 96, 4300, 110), NZ=8)


@jax.jit
def pallas_interleave_layers__ssm_conv_h3__geglu_ffn__prompt_kernel(
        A_q, A_k, A_v, A_shift_k, A_ssm_k, A_ssm_D, B_x, B_w_gate, B_w_up, B_w_down):
    _, S, D = A_q.shape
    F = B_w_gate.shape[1]
    KS = A_shift_k.shape[1]
    NB = S // TM
    P = S // B
    CH = (512, 512, 512, 256)
    assert sum(CH) == F and S % TM == 0 and NB >= 4 and D % 64 == 0 and KS == 4
    ft, fi = _dft_tables()
    to_ds = lambda x: jnp.swapaxes(x, 1, 2).reshape(D, S)
    hbm = pl.BlockSpec(memory_space=pl.ANY)
    blocks = pltpu.VMEM((NB, D, TM), BF16)
    out_t = pl.pallas_call(
        functools.partial(_kernel, D=D, F=F, NB=NB, KS=KS, CH=CH, cfg=_CFG),
        out_shape=jax.ShapeDtypeStruct((D, S), A_q.dtype),
        grid=(NB,),
        in_specs=[hbm] * 11,
        out_specs=hbm,
        scratch_shapes=[
            blocks,
            pltpu.VMEM((P - 1 + 2 * (P + PB) + 12, D, 2 * B), F32),
            pltpu.VMEM((D // 2, TM), U32),
            pltpu.VMEM((D // 2, PB * 2 * B), U32),
            pltpu.VMEM((D // 2, TM), U32),
            pltpu.VMEM((32, TM), F32),
            pltpu.VMEM((F, D), U32),
            pltpu.VMEM((D // 2, F), U32),
            pltpu.VMEM((D // 2, B), U32),
            pltpu.VMEM((F // 2, TM), U32),
            blocks, blocks, blocks, blocks,
            pltpu.VMEM((KS, D), BF16),
            pltpu.VMEM((D,), BF16),
            pltpu.VMEM((B, 2 * B), BF16),
            pltpu.VMEM((2 * B, B), BF16),
            pltpu.VMEM((D, F), BF16),
            pltpu.VMEM((D, F), BF16),
            pltpu.VMEM((D, F), BF16),
            pltpu.SemaphoreType.DMA((4 + 3 * len(CH) + 5 * NB,)),
        ],
        compiler_params=pltpu.CompilerParams(vmem_limit_bytes=100 * 2**20,
                                             dimension_semantics=("arbitrary",)),
    )(to_ds(A_q), to_ds(A_k), to_ds(A_v), A_ssm_k, A_shift_k.T, A_ssm_D,
      jnp.asarray(ft, BF16), jnp.asarray(fi, BF16), B_w_gate, B_w_up, B_w_down.T)
    return jnp.swapaxes(out_t.reshape(1, D, S), 1, 2)
```

```python
import functools

import numpy as np
import jax
import jax.numpy as jnp
from jax import lax
import jax.experimental.pallas as pl
import jax.experimental.pallas.tpu as pltpu

B = 128
PB = 2
TM = PB * B
UR = 16
GELU_C = 0.7978845608028654
EPS = 1e-5
F32 = jnp.float32
BF16 = jnp.bfloat16
U32 = jnp.uint32
_TN = (((0,), (0,)), ((), ()))


def _pack_rows(a):
    bits = np.asarray(a, np.float32).astype(jnp.bfloat16).view(np.uint16).astype(np.uint32)
    return bits[0::2] | (bits[1::2] << 16)


def _dft_tables():
    n = np.arange(B)[:, None]
    k = np.arange(B)[None, :]
    ang = 2.0 * np.pi * (((2 * k + 1) * n) % (4 * B)) / (4 * B)
    ft = np.concatenate([np.cos(ang), -np.sin(ang)], axis=1)
    return _pack_rows(ft), _pack_rows(ft.T / B)


def _gelu(x):
    inner = x * (GELU_C + (GELU_C * 0.044715) * (x * x))
    return (0.5 * x) * (1.0 + jnp.tanh(inner))


def _pack(x):
    return pltpu.bitcast(x, U32)


def _unpack(x):
    return pltpu.bitcast(x, BF16)


def _rsqrt_valu(x):
    i = lax.bitcast_convert_type(x, jnp.int32)
    y = lax.bitcast_convert_type(jnp.int32(0x5F3759DF) - lax.shift_right_logical(i, jnp.int32(1)), F32)
    hx = 0.5 * x
    for _ in range(4):
        y = y * (1.5 - hx * y * y)
    return y


def _stat_terms(x, y, pivot):
    a = x - pivot
    ay = a * y
    return a, a * a, ay, a * ay, ay * y, ay * ay


def _acc(accs, vals):
    return list(vals) if accs is None else [a + v for a, v in zip(accs, vals)]


def _stats(pivot, sums, y1, y2, ys, d, rsqrt):
    s1, s2, t1, t2, v1, v2 = [jnp.sum(t, axis=0, keepdims=True) for t in sums]
    inv = 1.0 / d
    m = s1 * inv
    e2 = s2 * inv
    r = rsqrt(jnp.maximum(e2 - m * m, 0.0) + EPS)
    mb = m + (r * (t1 - m * y1) * inv) * ys
    quad = (r * r * inv) * (v2 - 2.0 * m * v1 + m * m * y2)
    eb = e2 + ((2.0 * inv) * r * (t2 - m * t1)) * ys + (quad * ys) * ys
    r3 = rsqrt(jnp.maximum(eb - mb * mb, 0.0) + EPS)
    return pivot + m, r * ys, pivot + mb, r3


def _kernel(q_hbm, k_hbm, v_hbm, h_hbm, sk_hbm, d_hbm, ft_hbm, fi_hbm, wg_hbm, wu_hbm, wdt_hbm,
            o_hbm,
            ob, ug_ref, kv_ref, yf_ref, xn_ref, ys_ref, wt_ref, wd_ref, kp_ref, hh_ref,
            qb, kb, vb, hb, sk_ref, d_ref, ft_ref, fi_ref, wg_ref, wu_ref, wdt_ref,
            sem,
            *, D, F, NB, KS, CH, cfg):
    s = pl.program_id(0)
    P = NB * PB
    PAD = P - 1 - 2 * PB
    NC = len(CH)
    NU = D // UR
    NZ = cfg["NZ"]
    starts = [sum(CH[:i]) for i in range(NC)]
    lo, hi = slice(0, B), slice(B, 2 * B)

    UBASE = PAD
    HBASE = PAD + P + PB
    ZP = HBASE + P + PB
    KVD, CB, FENCE, YY, X1, X2, X3, YST = (ZP + i for i in (1, 2, 5, 6, 7, 8, 9, 10))

    zd = jnp.minimum(s, 0)

    Q, K, V, H = range(4)
    G, U, DW = range(3)

    def small_copy(i):
        src, dst = ((sk_hbm, sk_ref), (d_hbm, d_ref), (ft_hbm, ft_ref), (fi_hbm, fi_ref))[i]
        return pltpu.make_async_copy(src, dst, sem.at[i])

    def w_copy(i, c):
        src, dst = ((wg_hbm, wg_ref), (wu_hbm, wu_ref), (wdt_hbm, wdt_ref))[i]
        cs = pl.ds(starts[c], CH[c])
        return pltpu.make_async_copy(src.at[:, cs], dst.at[:, cs], sem.at[4 + i * NC + c])

    def blk_copy(i, b):
        src, dst = ((q_hbm, qb), (k_hbm, kb), (v_hbm, vb), (h_hbm, hb))[i]
        return pltpu.make_async_copy(src.at[:, pl.ds(b * TM, TM)], dst.at[b], sem.at[4 + 3 * NC + i * NB + b])

    def out_copy(b):
        start = b * TM if isinstance(b, int) else pl.multiple_of(b * TM, TM)
        return pltpu.make_async_copy(ob.at[b], o_hbm.at[:, pl.ds(start, TM)], sem.at[4 + 3 * NC + 4 * NB + b])

    def wait(*copies):
        for c in copies:
            c.wait()

    def init_taps():
        rows = lax.broadcasted_iota(jnp.int32, (16, D), 0)
        a = jnp.zeros((16, D), F32)
        skf = sk_ref[...].astype(F32)
        for j in range(KS):
            a = jnp.where(rows == j, jnp.broadcast_to(skf[j:j + 1, :], (16, D)), a)
        er = lax.broadcasted_iota(jnp.int32, (16, KS * B), 0)
        ec = lax.broadcasted_iota(jnp.int32, (16, KS * B), 1) // B
        e = jnp.where(er == ec, 1.0, 0.0).astype(BF16)
        t = lax.dot_general(a.astype(BF16), e, _TN, preferred_element_type=F32)
        for j in range(KS // 2):
            ug_ref[CB + j] = t[:, 2 * j * B:2 * (j + 1) * B]

    def init_d():
        rows = lax.broadcasted_iota(jnp.int32, (16, D), 0)
        a = jnp.where(rows == 0, jnp.broadcast_to(d_ref[...].astype(F32).reshape(1, D), (16, D)), 0.0)
        e = jnp.where(lax.broadcasted_iota(jnp.int32, (16, B), 0) == 0, 1.0, 0.0).astype(BF16)
        ug_ref[CB + 2, :, lo] = lax.dot_general(a.astype(BF16), e, _TN, preferred_element_type=F32)

    def kv_rows(r0, nr, parts, kr, vr, z):
        rs = slice(r0, r0 + nr)
        hs = slice(r0 // 2, (r0 + nr) // 2)
        lane = lax.broadcasted_iota(jnp.int32, (nr // 2, B), 1)
        taps = [ug_ref[CB + z + j // 2, rs, (lo, hi)[j % 2]] for j in range(KS)]
        dcol = ug_ref[CB + 2 + z, rs, lo]
        p = parts[0]
        kp = kp_ref[hs, :] if p == 0 else _pack(kr[rs, (p - 1) * B:p * B])
        for p in parts:
            ps = slice(p * B, (p + 1) * B)
            kcb = kr[rs, ps]
            kc = _pack(kcb)
            acc = kcb.astype(F32) * taps[0]
            for j in range(1, KS):
                sh = pltpu.roll(jnp.where(lane >= B - j, kp, kc), j, 1)
                acc = acc + _unpack(sh).astype(F32) * taps[j]
            kv_ref[hs, ps] = _pack((acc * vr[rs, ps].astype(F32)).astype(BF16))
            ug_ref[KVD, rs, ps] = _unpack(kv_ref[hs, ps]).astype(F32) * dcol
            kp = kc
        if parts[-1] == PB - 1:
            kp_ref[hs, :] = kp

    def fwd_h(hr, blk):
        for p in range(PB):
            ug_ref[HBASE + blk * PB + p] = jnp.dot(hr[:, p * B:(p + 1) * B], _unpack(ft_ref[...]),
                                                   preferred_element_type=F32)

    def fwd_u(blk):
        for p in range(PB):
            ug_ref[UBASE + blk * PB + p] = jnp.dot(_unpack(kv_ref[:, p * B:(p + 1) * B]), _unpack(ft_ref[...]),
                                                   preferred_element_type=F32)

    def mac_rows(r, nj, blk, chained):
        p0 = blk * PB
        rs = slice(r * 8, (r + 1) * 8)
        sgn = jnp.where(lax.broadcasted_iota(jnp.int32, (8, B), 1) % 2 == 0, 1.0, -1.0)
        static = isinstance(blk, int)
        z = zd if chained else 0
        ar = [None] * PB
        ai = [None] * PB
        us = {}
        for j in range(nj):
            gj = HBASE + (j + z if static else jnp.minimum(j, p0 + PB - 1))
            gr = ug_ref[gj, rs, lo]
            gi = ug_ref[gj, rs, hi]
            for p in range(PB):
                off = p - j
                if static and p0 + off < 0:
                    continue
                if off not in us:
                    ix = UBASE + p0 + off + (z if static else 0)
                    us[off] = (ug_ref[ix, rs, lo], ug_ref[ix, rs, hi])
                ur, ui = us[off]
                tr = ur * gr - ui * gi
                ti = ur * gi + ui * gr
                ar[p] = tr if ar[p] is None else ar[p] + tr
                ai[p] = ti if ai[p] is None else ai[p] + ti
            if chained and (j + 1) % cfg["JG"] == 0 and j + 1 < nj:
                for p in range(PB):
                    ug_ref[FENCE, p * 8:(p + 1) * 8, lo] = ar[p]
                    ug_ref[FENCE, p * 8:(p + 1) * 8, hi] = ai[p]
        zr = zi = None
        if not (static and blk == 0):
            zr, zi = ug_ref[ZP + z, rs, lo], ug_ref[ZP + z, rs, hi]
        out = []
        for p in range(PB):
            out.append((ar[p], ai[p]) if zr is None else (ar[p] - sgn * zi, ai[p] + sgn * zr))
            zr, zi = ar[p], ai[p]
        ug_ref[ZP, rs, lo] = zr
        ug_ref[ZP, rs, hi] = zi
        if chained:
            ug_ref[FENCE, 0:8, lo] = out[0][0]
            ug_ref[FENCE, 0:8, hi] = out[0][1]
        return out

    def mac(nj, blk, anchors):
        for g in range(NU):
            if anchors and g in anchors:
                ug_ref[FENCE, 0:8, lo] = anchors[g]
            res = [mac_rows(2 * g + i, nj, blk, anchors is not None) for i in range(2)]
            for p in range(PB):
                for i in range(2):
                    yf_ref[g * 8:(g + 1) * 8, (2 * p + i) * B:(2 * p + i + 1) * B] = _pack(
                        jnp.concatenate([x[p][i] for x in res], axis=0).astype(BF16))

    def inv_dot():
        for p in range(PB):
            for i in range(2):
                ug_ref[YST + i, :, p * B:(p + 1) * B] = jnp.dot(
                    _unpack(yf_ref[:, (2 * p + i) * B:(2 * p + i + 1) * B]), _unpack(fi_ref[i * B // 2:(i + 1) * B // 2, :]),
                    preferred_element_type=F32)

    def side_post(old, qr, kr, vr, anchors, zero_fill=False):
        chained = anchors is not None
        z = zd if chained else 0
        pivot = qr[0:16, :].astype(F32)[0:1]
        pb = jnp.broadcast_to(pivot, (8, TM))
        accs = None
        for g in range(NU):
            rs = slice(g * UR, (g + 1) * UR)
            if chained:
                ug_ref[FENCE, 8:16, lo] = anchors[g]
                x = ug_ref[X2 + z, rs, :]
                ug_ref[X3, rs, :] = x + (x - old[0]) * old[1] * ug_ref[YY + z, rs, :]
            x = qr[rs, :].astype(F32)
            y = ug_ref[YST + z, rs, :] + ug_ref[YST + 1 + z, rs, :] + ug_ref[KVD + z, rs, :]
            ug_ref[YY, rs, :] = y
            for i in range(UR // 8):
                yi = y[i * 8:(i + 1) * 8]
                accs = _acc(accs, _stat_terms(x[i * 8:(i + 1) * 8], yi, pb) + (yi, yi * yi))
            if chained:
                kv_rows(g * UR, UR, (0,), kr, vr, z)
            if zero_fill:
                for i in range(NZ, (NZ + PAD) // 2):
                    ug_ref[i + z, rs, :] = jnp.zeros((UR, 2 * B), F32)
        rsqrt = _rsqrt_valu if chained else lax.rsqrt
        y1 = jnp.sum(accs[6], axis=0, keepdims=True)
        y2 = jnp.sum(accs[7], axis=0, keepdims=True)
        ms = y2 * (1.0 / D) + 1e-30
        sy = rsqrt(ms)
        ys_ref[0:1, :] = y1 * sy
        ys_ref[8:9, :] = (y2 * sy) * sy
        ys_ref[16:17, :] = ms * sy
        mu, r, mu3, r3 = _stats(pivot, accs[:6], y1, y2, 1.0, D, rsqrt)
        for g in range(NU):
            rs = slice(g * UR, (g + 1) * UR)
            if chained:
                ug_ref[FENCE, 8:16, lo] = anchors[NU + g]
            x = qr[rs, :].astype(F32)
            y = ug_ref[YY + z, rs, :]
            xo = x + (x - mu) * r * y
            xn = (xo - mu3) * r3
            xn_ref[g * UR // 2:(g + 1) * UR // 2, :] = _pack(xn.astype(BF16))
            ug_ref[YY, rs, :] = y * sy
            ug_ref[X1, rs, :] = xo
            if chained:
                ug_ref[FENCE, 0:8, lo] = xn[UR - 8:UR, hi]
                kv_rows(g * UR, UR, (1,), kr, vr, z)
            if zero_fill:
                for i in range((NZ + PAD) // 2, PAD):
                    ug_ref[i + z, rs, :] = jnp.zeros((UR, 2 * B), F32)

    def gu_rows(f0, fc, xn):
        return jnp.dot(_unpack(wt_ref[f0:f0 + fc, :]), xn, preferred_element_type=F32)

    def gu(c, xn):
        return gu_rows(starts[c], CH[c], xn)

    def gu_first(c, n_now, xn):
        f0, fc = starts[c], CH[c]
        pieces = []
        for f in range(f0, f0 + fc, B):
            gt = wg_ref[:, f:f + B].T
            ut = wu_ref[:, f:f + B].T
            pieces += [t[16 * i:16 * (i + 1)] for i in range(B // 16) for t in (gt, ut)]
        lhs = jnp.concatenate(pieces, axis=0)
        wt_ref[f0:f0 + fc, :] = _pack(lhs)
        return jnp.dot(lhs[0:2 * n_now], xn, preferred_element_type=F32)

    def act(r, f0):
        for i in range(r.shape[0] // 32):
            h16 = (_gelu(r[32 * i:32 * i + 16]) * r[32 * i + 16:32 * i + 32]).astype(BF16)
            hh_ref[f0 // 2 + 8 * i:f0 // 2 + 8 * (i + 1), :] = _pack(h16)

    def dn(c, acc, first=False):
        f0, fc = starts[c], CH[c]
        if first:
            w = wdt_ref[:, f0:f0 + fc]
            wd_ref[:, f0:f0 + fc] = _pack(w)
        else:
            w = _unpack(wd_ref[:, f0:f0 + fc])
        return jnp.dot(w, _unpack(hh_ref[f0 // 2:(f0 + fc) // 2, :]), preferred_element_type=F32) + acc

    def mlp(xn, acc, side, res_slot, r0=None):
        raws = [gu(0, xn) if r0 is None else r0, gu(1, xn)]
        seq = raws[(r0 is not None):]
        for c in range(NC - 1):
            if c >= 1:
                raws.append(gu(c + 1, xn))
                seq.append(raws[-1])
            if c > 0 or r0 is None:
                act(raws[c], starts[c])
            acc = dn(c, acc)
            seq.append(acc)
        side(seq)
        if res_slot is not None:
            acc = acc + ug_ref[res_slot]
        act(raws[NC - 1], starts[NC - 1])
        return dn(NC - 1, acc)

    def paced(seq, n_units, t0, dt, t1=None, dt1=None):
        anchors = {}
        for u in range(n_units):
            t = t0 + dt * u
            if t1 is not None and u >= n_units // 2:
                t = t1 + dt1 * (u - n_units // 2)
            for val in seq:
                n = val.shape[0]
                if t < PB * n:
                    r = (t % n) // 8 * 8
                    anchors[u] = val[r:r + 8, (lo, hi)[t // n]]
                    break
                t -= PB * n
        return anchors

    def mid_norm(x2):
        ug_ref[X2] = x2
        st = []
        for p in range(PB):
            ps = slice(p * B, (p + 1) * B)
            pivot = x2[0:1, ps]
            pb = jnp.broadcast_to(pivot, (8, B))
            accs = None
            for i in range(D // 8):
                rs = slice(i * 8, (i + 1) * 8)
                accs = _acc(accs, _stat_terms(x2[rs, ps], ug_ref[YY, rs, ps], pb))
            st.append(_stats(pivot, accs, ys_ref[0:1, ps], ys_ref[8:9, ps], ys_ref[16:17, ps], D, lax.rsqrt))
        mu, r, mu3, r3 = [jnp.concatenate([st[p][i] for p in range(PB)], axis=1) for i in range(4)]
        dr = D - cfg["DR"]
        x2h = jnp.concatenate([ug_ref[X2, 0:dr, hi], ug_ref[X2 + zd, dr:D, hi]], axis=0)
        x2r = jnp.concatenate([ug_ref[X2, :, lo], x2h], axis=1)
        xn3 = ((x2r + (x2r - mu) * r * ug_ref[YY] - mu3) * r3).astype(BF16)
        return xn3, (mu, r)

    def emit(x4, b):
        ob[b] = x4.astype(ob.dtype)
        out_copy(b).start()

    zeros = lambda: jnp.zeros((D, TM), F32)

    @pl.when(s == 0)
    def _():
        hb_ = cfg["HOLD"]
        order = [small_copy(0), blk_copy(K, 0), blk_copy(V, 0), small_copy(1), small_copy(2), small_copy(3),
                 blk_copy(H, 0), blk_copy(Q, 0)]
        order += [w_copy(i, c) for c in range(3) for i in (G, U)]
        order += [w_copy(DW, 0), w_copy(G, 3), w_copy(U, 3), w_copy(DW, 1), w_copy(DW, 2), w_copy(DW, 3)]
        order += [blk_copy(i, 1) for i in (K, V, H, Q)] + [blk_copy(i, 2) for i in (K, V)]
        late = [blk_copy(H, 2), blk_copy(Q, 2)] + [blk_copy(i, b) for b in range(3, NB) for i in (K, V, H, Q)]
        for c in order:
            c.start()
        kp_ref[...] = jnp.zeros(kp_ref.shape, U32)
        ug_ref[0:NZ] = jnp.zeros((NZ, D, 2 * B), F32)

        wait(small_copy(0))
        init_taps()

        wait(blk_copy(K, 0), blk_copy(V, 0), small_copy(1), small_copy(2))
        init_d()
        kv_rows(0, D, (0, 1), kb.at[0], vb.at[0], 0)
        fwd_u(0)

        wait(small_copy(3), blk_copy(H, 0), blk_copy(Q, 0))
        fwd_h(hb.at[0], 0)
        mac(PB, 0, None)
        inv_dot()
        side_post(None, qb.at[0], None, None, None)

        wait(w_copy(G, 0), w_copy(U, 0))
        xn = _unpack(xn_ref[...])
        act(gu_first(0, CH[0] - hb_, xn), starts[0])

        wait(w_copy(G, 1), w_copy(U, 1))
        for c in late:
            c.start()
        act(gu_rows(starts[1] - hb_, hb_, xn), starts[1] - hb_)
        act(gu_first(1, CH[1] - hb_, xn), starts[1])

        wait(w_copy(G, 2), w_copy(U, 2))
        act(gu_rows(starts[2] - hb_, hb_, xn), starts[2] - hb_)
        act(gu_first(2, CH[2] - hb_, xn), starts[2])

        wait(w_copy(DW, 0), w_copy(G, 3), w_copy(U, 3), w_copy(DW, 1))
        act(gu_rows(starts[3] - hb_, hb_, xn), starts[3] - hb_)
        acc = dn(0, ug_ref[X1], True)
        act(gu_first(3, CH[3], xn), starts[3])
        acc = dn(1, acc, True)

        wait(w_copy(DW, 2), w_copy(DW, 3), blk_copy(K, 1), blk_copy(V, 1), blk_copy(H, 1))
        acc = dn(2, acc, True)
        anchors = paced([acc], NU, 0, 30)
        for g in range(NU):
            ug_ref[FENCE, 0:8, lo] = anchors[g]
            kv_rows(g * UR, UR, (0, 1), kb.at[1], vb.at[1], zd)
        x2 = dn(3, acc, True)
        fwd_h(hb.at[1], 1)
        fwd_u(1)
        xn3, old = mid_norm(x2)
        r0 = gu(0, xn3)
        mac(2 * PB, 1, paced([r0], NU, 0, 64))
        act(r0, starts[0])

        wait(blk_copy(Q, 1), blk_copy(K, 2), blk_copy(V, 2))
        inv_dot()
        side = lambda seq: side_post(old, qb.at[1], kb.at[2], vb.at[2], paced(seq, 2 * NU, *cfg["FP"]), True)
        emit(mlp(xn3, zeros(), side, X3, r0), 0)
        wait(*late)

    @pl.when(s > 0)
    def _():
        n1 = jnp.minimum(s + 1, NB - 1)
        n2 = jnp.minimum(s + 2, NB - 1)
        fwd_h(hb.at[n1], s + 1)
        fwd_u(s + 1)

        def side1(seq):
            ends = [v[v.shape[0] - 8:, t] for v in seq[:2] for t in (lo, hi)]
            anchors = {0: seq[0][0:8, lo]}
            anchors.update(zip(cfg["AG"], ends))
            mac(P, s + 1, anchors)

        x2 = mlp(_unpack(xn_ref[...]), ug_ref[X1], side1, None)
        inv_dot()
        xn3, old = mid_norm(x2)
        side2 = lambda seq: side_post(old, qb.at[n1], kb.at[n2], vb.at[n2], paced(seq, 2 * NU, *cfg["SP"]))
        emit(mlp(xn3, zeros(), side2, X3), s)

    @pl.when(s == NB - 1)
    def _():
        wait(*[out_copy(b) for b in range(NB)])


_CFG = dict(JG=4, AG=(6, 10, 14), HOLD=128, DR=128,
            SP=(1000, 64, 5700, 72), FP=(64, 96, 4300, 110), NZ=8)


@jax.jit
def pallas_interleave_layers__ssm_conv_h3__geglu_ffn__prompt_kernel(
        A_q, A_k, A_v, A_shift_k, A_ssm_k, A_ssm_D, B_x, B_w_gate, B_w_up, B_w_down):
    _, S, D = A_q.shape
    F = B_w_gate.shape[1]
    KS = A_shift_k.shape[1]
    NB = S // TM
    P = S // B
    CH = (512, 512, 512, 256)
    assert sum(CH) == F and S % TM == 0 and NB >= 4 and D % 64 == 0 and KS == 4
    ft, fi = _dft_tables()
    to_ds = lambda x: jnp.swapaxes(x, 1, 2).reshape(D, S)
    hbm = pl.BlockSpec(memory_space=pl.ANY)
    blocks = pltpu.VMEM((NB, D, TM), BF16)
    out_t = pl.pallas_call(
        functools.partial(_kernel, D=D, F=F, NB=NB, KS=KS, CH=CH, cfg=_CFG),
        out_shape=jax.ShapeDtypeStruct((D, S), A_q.dtype),
        grid=(NB,),
        in_specs=[hbm] * 11,
        out_specs=hbm,
        scratch_shapes=[
            blocks,
            pltpu.VMEM((P - 1 - 2 * PB + 2 * (P + PB) + 12, D, 2 * B), F32),
            pltpu.VMEM((D // 2, TM), U32),
            pltpu.VMEM((D // 2, PB * 2 * B), U32),
            pltpu.VMEM((D // 2, TM), U32),
            pltpu.VMEM((32, TM), F32),
            pltpu.VMEM((F, D), U32),
            pltpu.VMEM((D // 2, F), U32),
            pltpu.VMEM((D // 2, B), U32),
            pltpu.VMEM((F // 2, TM), U32),
            blocks, blocks, blocks, blocks,
            pltpu.VMEM((KS, D), BF16),
            pltpu.VMEM((D,), BF16),
            pltpu.VMEM((B // 2, 2 * B), U32),
            pltpu.VMEM((B, B), U32),
            pltpu.VMEM((D, F), BF16),
            pltpu.VMEM((D, F), BF16),
            pltpu.VMEM((D, F), BF16),
            pltpu.SemaphoreType.DMA((4 + 3 * len(CH) + 5 * NB,)),
        ],
        compiler_params=pltpu.CompilerParams(vmem_limit_bytes=100 * 2**20,
                                             dimension_semantics=("arbitrary",)),
    )(to_ds(A_q), to_ds(A_k), to_ds(A_v), A_ssm_k, A_shift_k.T, A_ssm_D,
      jnp.asarray(ft), jnp.asarray(fi), B_w_gate, B_w_up, B_w_down.T)
    return jnp.swapaxes(out_t.reshape(1, D, S), 1, 2)
```

```python
import functools

import numpy as np
import jax
import jax.numpy as jnp
from jax import lax
import jax.experimental.pallas as pl
import jax.experimental.pallas.tpu as pltpu

B = 128
PB = 2
TM = PB * B
UR = 16
GELU_C = 0.7978845608028654
EPS = 1e-5
F32 = jnp.float32
BF16 = jnp.bfloat16
U32 = jnp.uint32
_TN = (((0,), (0,)), ((), ()))


def _pack_rows(a):
    bits = np.asarray(a, np.float32).astype(jnp.bfloat16).view(np.uint16).astype(np.uint32)
    return bits[0::2] | (bits[1::2] << 16)


def _dft_tables():
    n = np.arange(B)[:, None]
    k = np.arange(B)[None, :]
    ang = 2.0 * np.pi * (((2 * k + 1) * n) % (4 * B)) / (4 * B)
    ft = np.concatenate([np.cos(ang), -np.sin(ang)], axis=1)
    return _pack_rows(ft), _pack_rows(ft.T / B)


def _gelu(x):
    inner = x * (GELU_C + (GELU_C * 0.044715) * (x * x))
    return (0.5 * x) * (1.0 + jnp.tanh(inner))


def _pack(x):
    return pltpu.bitcast(x, U32)


def _unpack(x):
    return pltpu.bitcast(x, BF16)


def _rsqrt_valu(x):
    i = lax.bitcast_convert_type(x, jnp.int32)
    y = lax.bitcast_convert_type(jnp.int32(0x5F3759DF) - lax.shift_right_logical(i, jnp.int32(1)), F32)
    hx = 0.5 * x
    for _ in range(4):
        y = y * (1.5 - hx * y * y)
    return y


def _stat_terms(x, y, pivot):
    a = x - pivot
    ay = a * y
    return a, a * a, ay, a * ay, ay * y, ay * ay


def _acc(accs, vals):
    return list(vals) if accs is None else [a + v for a, v in zip(accs, vals)]


def _stats(pivot, sums, y1, y2, ys, d, rsqrt):
    s1, s2, t1, t2, v1, v2 = [jnp.sum(t, axis=0, keepdims=True) for t in sums]
    inv = 1.0 / d
    m = s1 * inv
    e2 = s2 * inv
    r = rsqrt(jnp.maximum(e2 - m * m, 0.0) + EPS)
    mb = m + (r * (t1 - m * y1) * inv) * ys
    quad = (r * r * inv) * (v2 - 2.0 * m * v1 + m * m * y2)
    eb = e2 + ((2.0 * inv) * r * (t2 - m * t1)) * ys + (quad * ys) * ys
    r3 = rsqrt(jnp.maximum(eb - mb * mb, 0.0) + EPS)
    return pivot + m, r * ys, pivot + mb, r3


def _kernel(q_hbm, k_hbm, v_hbm, h_hbm, sk_hbm, d_hbm, ft_hbm, fi_hbm, wg_hbm, wu_hbm, wdt_hbm,
            o_hbm,
            ob, ug_ref, kv_ref, yf_ref, xn_ref, ys_ref, wt_ref, wd_ref, kp_ref, hh_ref,
            qb, kb, vb, hb, sk_ref, d_ref, ft_ref, fi_ref, wg_ref, wu_ref, wdt_ref,
            sem,
            *, D, F, NB, KS, CH, cfg):
    s = pl.program_id(0)
    P = NB * PB
    PAD = P - 1 - 2 * PB
    NC = len(CH)
    NU = D // UR
    NZ = cfg["NZ"]
    starts = [sum(CH[:i]) for i in range(NC)]
    lo, hi = slice(0, B), slice(B, 2 * B)

    UBASE = PAD
    HBASE = PAD + P
    ZP = HBASE + P
    KVD, CB, FENCE, YY, X1, X2, X3, YST = (ZP + i for i in (1, 2, 5, 6, 7, 8, 9, 10))

    zd = jnp.minimum(s, 0)

    Q, K, V, H = range(4)
    G, U, DW = range(3)

    def small_copy(i):
        src, dst = ((sk_hbm, sk_ref), (d_hbm, d_ref), (ft_hbm, ft_ref), (fi_hbm, fi_ref))[i]
        return pltpu.make_async_copy(src, dst, sem.at[i])

    def w_copy(i, c):
        src, dst = ((wg_hbm, wg_ref), (wu_hbm, wu_ref), (wdt_hbm, wdt_ref))[i]
        cs = pl.ds(starts[c], CH[c])
        return pltpu.make_async_copy(src.at[:, cs], dst.at[:, cs], sem.at[4 + i * NC + c])

    def blk_copy(i, b):
        src, dst = ((q_hbm, qb), (k_hbm, kb), (v_hbm, vb), (h_hbm, hb))[i]
        return pltpu.make_async_copy(src.at[:, pl.ds(b * TM, TM)], dst.at[b], sem.at[4 + 3 * NC + i * NB + b])

    def out_copy(b):
        start = b * TM if isinstance(b, int) else pl.multiple_of(b * TM, TM)
        return pltpu.make_async_copy(ob.at[b], o_hbm.at[:, pl.ds(start, TM)], sem.at[4 + 3 * NC + 4 * NB + b])

    def wait(*copies):
        for c in copies:
            c.wait()

    def init_taps():
        rows = lax.broadcasted_iota(jnp.int32, (16, D), 0)
        a = jnp.zeros((16, D), F32)
        skf = sk_ref[...].astype(F32)
        for j in range(KS):
            a = jnp.where(rows == j, jnp.broadcast_to(skf[j:j + 1, :], (16, D)), a)
        er = lax.broadcasted_iota(jnp.int32, (16, KS * B), 0)
        ec = lax.broadcasted_iota(jnp.int32, (16, KS * B), 1) // B
        e = jnp.where(er == ec, 1.0, 0.0).astype(BF16)
        t = lax.dot_general(a.astype(BF16), e, _TN, preferred_element_type=F32)
        for j in range(KS // 2):
            ug_ref[CB + j] = t[:, 2 * j * B:2 * (j + 1) * B]

    def init_d():
        rows = lax.broadcasted_iota(jnp.int32, (16, D), 0)
        a = jnp.where(rows == 0, jnp.broadcast_to(d_ref[...].astype(F32).reshape(1, D), (16, D)), 0.0)
        e = jnp.where(lax.broadcasted_iota(jnp.int32, (16, B), 0) == 0, 1.0, 0.0).astype(BF16)
        ug_ref[CB + 2, :, lo] = lax.dot_general(a.astype(BF16), e, _TN, preferred_element_type=F32)

    def kv_rows(r0, nr, parts, kr, vr, z):
        rs = slice(r0, r0 + nr)
        hs = slice(r0 // 2, (r0 + nr) // 2)
        lane = lax.broadcasted_iota(jnp.int32, (nr // 2, B), 1)
        taps = [ug_ref[CB + z + j // 2, rs, (lo, hi)[j % 2]] for j in range(KS)]
        dcol = ug_ref[CB + 2 + z, rs, lo]
        p = parts[0]
        kp = kp_ref[hs, :] if p == 0 else _pack(kr[rs, (p - 1) * B:p * B])
        for p in parts:
            ps = slice(p * B, (p + 1) * B)
            kcb = kr[rs, ps]
            kc = _pack(kcb)
            acc = kcb.astype(F32) * taps[0]
            for j in range(1, KS):
                sh = pltpu.roll(jnp.where(lane >= B - j, kp, kc), j, 1)
                acc = acc + _unpack(sh).astype(F32) * taps[j]
            kv_ref[hs, ps] = _pack((acc * vr[rs, ps].astype(F32)).astype(BF16))
            ug_ref[KVD, rs, ps] = _unpack(kv_ref[hs, ps]).astype(F32) * dcol
            kp = kc
        if parts[-1] == PB - 1:
            kp_ref[hs, :] = kp

    def fwd_h(hr, blk):
        for p in range(PB):
            ug_ref[HBASE + blk * PB + p] = jnp.dot(hr[:, p * B:(p + 1) * B], _unpack(ft_ref[...]),
                                                   preferred_element_type=F32)

    def fwd_u(blk):
        for p in range(PB):
            ug_ref[UBASE + blk * PB + p] = jnp.dot(_unpack(kv_ref[:, p * B:(p + 1) * B]), _unpack(ft_ref[...]),
                                                   preferred_element_type=F32)

    def mac_rows(r, nj, blk, chained):
        p0 = blk * PB
        rs = slice(r * 8, (r + 1) * 8)
        sgn = jnp.where(lax.broadcasted_iota(jnp.int32, (8, B), 1) % 2 == 0, 1.0, -1.0)
        static = isinstance(blk, int)
        z = zd if chained else 0
        ar = [None] * PB
        ai = [None] * PB
        us = {}
        for j in range(nj):
            gj = HBASE + (j + z if static else jnp.minimum(j, p0 + PB - 1))
            gr = ug_ref[gj, rs, lo]
            gi = ug_ref[gj, rs, hi]
            for p in range(PB):
                off = p - j
                if static and p0 + off < 0:
                    continue
                if off not in us:
                    ix = UBASE + p0 + off + (z if static else 0)
                    us[off] = (ug_ref[ix, rs, lo], ug_ref[ix, rs, hi])
                ur, ui = us[off]
                tr = ur * gr - ui * gi
                ti = ur * gi + ui * gr
                ar[p] = tr if ar[p] is None else ar[p] + tr
                ai[p] = ti if ai[p] is None else ai[p] + ti
            if chained and (j + 1) % cfg["JG"] == 0 and j + 1 < nj:
                for p in range(PB):
                    ug_ref[FENCE, p * 8:(p + 1) * 8, lo] = ar[p]
                    ug_ref[FENCE, p * 8:(p + 1) * 8, hi] = ai[p]
        zr = zi = None
        if not (static and blk == 0):
            zr, zi = ug_ref[ZP + z, rs, lo], ug_ref[ZP + z, rs, hi]
        out = []
        for p in range(PB):
            out.append((ar[p], ai[p]) if zr is None else (ar[p] - sgn * zi, ai[p] + sgn * zr))
            zr, zi = ar[p], ai[p]
        ug_ref[ZP, rs, lo] = zr
        ug_ref[ZP, rs, hi] = zi
        if chained:
            ug_ref[FENCE, 0:8, lo] = out[0][0]
            ug_ref[FENCE, 0:8, hi] = out[0][1]
        return out

    def mac(nj, blk, anchors):
        for g in range(NU):
            if anchors and g in anchors:
                ug_ref[FENCE, 0:8, lo] = anchors[g]
            res = [mac_rows(2 * g + i, nj, blk, anchors is not None) for i in range(2)]
            for p in range(PB):
                for i in range(2):
                    yf_ref[g * 8:(g + 1) * 8, (2 * p + i) * B:(2 * p + i + 1) * B] = _pack(
                        jnp.concatenate([x[p][i] for x in res], axis=0).astype(BF16))

    def inv_dot():
        for p in range(PB):
            for i in range(2):
                ug_ref[YST + i, :, p * B:(p + 1) * B] = jnp.dot(
                    _unpack(yf_ref[:, (2 * p + i) * B:(2 * p + i + 1) * B]),
                    _unpack(fi_ref[i * B // 2:(i + 1) * B // 2, :]), preferred_element_type=F32)

    def side_post(old, qr, kr, vr, anchors, zero_fill=False):
        chained = anchors is not None
        z = zd if chained else 0
        pivot = qr[0:16, :].astype(F32)[0:1]
        pb = jnp.broadcast_to(pivot, (8, TM))
        accs = None
        for g in range(NU):
            rs = slice(g * UR, (g + 1) * UR)
            if chained:
                ug_ref[FENCE, 8:16, lo] = anchors[g]
                x = ug_ref[X2 + z, rs, :]
                ug_ref[X3, rs, :] = x + (x - old[0]) * old[1] * ug_ref[YY + z, rs, :]
            x = qr[rs, :].astype(F32)
            y = ug_ref[YST + z, rs, :] + ug_ref[YST + 1 + z, rs, :] + ug_ref[KVD + z, rs, :]
            ug_ref[YY, rs, :] = y
            for i in range(UR // 8):
                yi = y[i * 8:(i + 1) * 8]
                accs = _acc(accs, _stat_terms(x[i * 8:(i + 1) * 8], yi, pb) + (yi, yi * yi))
            if chained:
                kv_rows(g * UR, UR, (0,), kr, vr, z)
            if zero_fill:
                for i in range(NZ, (NZ + PAD) // 2):
                    ug_ref[i + z, rs, :] = jnp.zeros((UR, 2 * B), F32)
        rsqrt = _rsqrt_valu if chained else lax.rsqrt
        y1 = jnp.sum(accs[6], axis=0, keepdims=True)
        y2 = jnp.sum(accs[7], axis=0, keepdims=True)
        ms = y2 * (1.0 / D) + 1e-30
        sy = rsqrt(ms)
        ys_ref[0:1, :] = y1 * sy
        ys_ref[8:9, :] = (y2 * sy) * sy
        ys_ref[16:17, :] = ms * sy
        mu, r, mu3, r3 = _stats(pivot, accs[:6], y1, y2, 1.0, D, rsqrt)
        for g in range(NU):
            rs = slice(g * UR, (g + 1) * UR)
            if chained:
                ug_ref[FENCE, 8:16, lo] = anchors[NU + g]
            x = qr[rs, :].astype(F32)
            y = ug_ref[YY + z, rs, :]
            xo = x + (x - mu) * r * y
            xn = (xo - mu3) * r3
            xn_ref[g * UR // 2:(g + 1) * UR // 2, :] = _pack(xn.astype(BF16))
            ug_ref[YY, rs, :] = y * sy
            ug_ref[X1, rs, :] = xo
            if chained:
                ug_ref[FENCE, 0:8, lo] = xn[UR - 8:UR, hi]
                kv_rows(g * UR, UR, (1,), kr, vr, z)
            if zero_fill:
                for i in range((NZ + PAD) // 2, PAD):
                    ug_ref[i + z, rs, :] = jnp.zeros((UR, 2 * B), F32)

    def gu_rows(f0, fc, xn):
        return jnp.dot(_unpack(wt_ref[f0:f0 + fc, :]), xn, preferred_element_type=F32)

    def gu(c, xn):
        return gu_rows(starts[c], CH[c], xn)

    def gu_first(c, n_now, xn):
        f0, fc = starts[c], CH[c]
        pieces = []
        for f in range(f0, f0 + fc, B):
            gt = wg_ref[:, f:f + B].T
            ut = wu_ref[:, f:f + B].T
            pieces += [t[16 * i:16 * (i + 1)] for i in range(B // 16) for t in (gt, ut)]
        lhs = jnp.concatenate(pieces, axis=0)
        wt_ref[f0:f0 + fc, :] = _pack(lhs)
        return jnp.dot(lhs[0:2 * n_now], xn, preferred_element_type=F32)

    def act(r, f0):
        for i in range(r.shape[0] // 32):
            h16 = (_gelu(r[32 * i:32 * i + 16]) * r[32 * i + 16:32 * i + 32]).astype(BF16)
            hh_ref[f0 // 2 + 8 * i:f0 // 2 + 8 * (i + 1), :] = _pack(h16)

    def dn(c, acc, first=False):
        f0, fc = starts[c], CH[c]
        if first:
            w = wdt_ref[:, f0:f0 + fc]
            wd_ref[:, f0:f0 + fc] = _pack(w)
        else:
            w = _unpack(wd_ref[:, f0:f0 + fc])
        return jnp.dot(w, _unpack(hh_ref[f0 // 2:(f0 + fc) // 2, :]), preferred_element_type=F32) + acc

    def mlp(xn, acc, side, res_slot, r0=None):
        raws = [gu(0, xn) if r0 is None else r0, gu(1, xn)]
        seq = raws[(r0 is not None):]
        for c in range(NC - 1):
            if c >= 1:
                raws.append(gu(c + 1, xn))
                seq.append(raws[-1])
            if c > 0 or r0 is None:
                act(raws[c], starts[c])
            acc = dn(c, acc)
            seq.append(acc)
        side(seq)
        if res_slot is not None:
            acc = acc + ug_ref[res_slot]
        act(raws[NC - 1], starts[NC - 1])
        return dn(NC - 1, acc)

    def paced(seq, n_units, t0, dt, t1=None, dt1=None):
        anchors = {}
        for u in range(n_units):
            t = t0 + dt * u
            if t1 is not None and u >= n_units // 2:
                t = t1 + dt1 * (u - n_units // 2)
            for val in seq:
                n = val.shape[0]
                if t < PB * n:
                    r = (t % n) // 8 * 8
                    anchors[u] = val[r:r + 8, (lo, hi)[t // n]]
                    break
                t -= PB * n
        return anchors

    def mid_norm(x2):
        ug_ref[X2] = x2
        st = []
        for p in range(PB):
            ps = slice(p * B, (p + 1) * B)
            pivot = x2[0:1, ps]
            pb = jnp.broadcast_to(pivot, (8, B))
            accs = None
            for i in range(D // 8):
                rs = slice(i * 8, (i + 1) * 8)
                accs = _acc(accs, _stat_terms(x2[rs, ps], ug_ref[YY, rs, ps], pb))
            st.append(_stats(pivot, accs, ys_ref[0:1, ps], ys_ref[8:9, ps], ys_ref[16:17, ps], D, lax.rsqrt))
        mu, r, mu3, r3 = [jnp.concatenate([st[p][i] for p in range(PB)], axis=1) for i in range(4)]
        dr = D - cfg["DR"]
        x2h = jnp.concatenate([ug_ref[X2, 0:dr, hi], ug_ref[X2 + zd, dr:D, hi]], axis=0)
        x2r = jnp.concatenate([ug_ref[X2, :, lo], x2h], axis=1)
        xn3 = ((x2r + (x2r - mu) * r * ug_ref[YY] - mu3) * r3).astype(BF16)
        return xn3, (mu, r)

    def emit(x4, b):
        ob[b] = x4.astype(ob.dtype)
        out_copy(b).start()

    zeros = lambda: jnp.zeros((D, TM), F32)

    @pl.when(s == 0)
    def _():
        hb_ = cfg["HOLD"]
        order = [small_copy(0), blk_copy(K, 0), blk_copy(V, 0), small_copy(1), small_copy(2), small_copy(3),
                 blk_copy(H, 0), blk_copy(Q, 0)]
        order += [w_copy(i, c) for c in range(3) for i in (G, U)]
        order += [w_copy(DW, 0), w_copy(G, 3), w_copy(U, 3), w_copy(DW, 1), w_copy(DW, 2), w_copy(DW, 3)]
        order += [blk_copy(i, 1) for i in (K, V, H, Q)] + [blk_copy(i, 2) for i in (K, V)]
        late = [blk_copy(H, 2), blk_copy(Q, 2)] + [blk_copy(i, b) for b in range(3, NB) for i in (K, V, H, Q)]
        for c in order:
            c.start()
        kp_ref[...] = jnp.zeros(kp_ref.shape, U32)

        @pl.loop(0, NZ)
        def _(i):
            ug_ref[i] = jnp.zeros((D, 2 * B), F32)

        wait(small_copy(0))
        init_taps()

        wait(blk_copy(K, 0), blk_copy(V, 0), small_copy(1), small_copy(2))
        init_d()
        kv_rows(0, D, (0, 1), kb.at[0], vb.at[0], 0)
        fwd_u(0)

        wait(small_copy(3), blk_copy(H, 0), blk_copy(Q, 0))
        fwd_h(hb.at[0], 0)
        mac(PB, 0, None)
        inv_dot()
        side_post(None, qb.at[0], None, None, None)

        wait(w_copy(G, 0), w_copy(U, 0))
        xn = _unpack(xn_ref[...])
        act(gu_first(0, CH[0] - hb_, xn), starts[0])

        wait(w_copy(G, 1), w_copy(U, 1))
        for c in late:
            c.start()
        act(gu_rows(starts[1] - hb_, hb_, xn), starts[1] - hb_)
        act(gu_first(1, CH[1] - hb_, xn), starts[1])

        wait(w_copy(G, 2), w_copy(U, 2))
        act(gu_rows(starts[2] - hb_, hb_, xn), starts[2] - hb_)
        act(gu_first(2, CH[2] - hb_, xn), starts[2])

        wait(w_copy(DW, 0), w_copy(G, 3), w_copy(U, 3), w_copy(DW, 1))
        act(gu_rows(starts[3] - hb_, hb_, xn), starts[3] - hb_)
        acc = dn(0, ug_ref[X1], True)
        act(gu_first(3, CH[3], xn), starts[3])
        acc = dn(1, acc, True)

        wait(w_copy(DW, 2), w_copy(DW, 3), blk_copy(K, 1), blk_copy(V, 1), blk_copy(H, 1))
        acc = dn(2, acc, True)
        anchors = paced([acc], NU, 0, 30)
        for g in range(NU):
            ug_ref[FENCE, 0:8, lo] = anchors[g]
            kv_rows(g * UR, UR, (0, 1), kb.at[1], vb.at[1], zd)
        x2 = dn(3, acc, True)
        fwd_h(hb.at[1], 1)
        fwd_u(1)
        xn3, old = mid_norm(x2)
        r0 = gu(0, xn3)
        mac(2 * PB, 1, paced([r0], NU, 0, 64))
        act(r0, starts[0])

        wait(blk_copy(Q, 1), blk_copy(K, 2), blk_copy(V, 2))
        inv_dot()
        side = lambda seq: side_post(old, qb.at[1], kb.at[2], vb.at[2], paced(seq, 2 * NU, *cfg["FP"]), True)
        emit(mlp(xn3, zeros(), side, X3, r0), 0)
        wait(*late)

    @pl.when(jnp.logical_and(s > 0, s < NB - 1))
    def _():
        n1 = s + 1
        n2 = jnp.minimum(s + 2, NB - 1)
        fwd_h(hb.at[n1], s + 1)
        fwd_u(s + 1)

        def side1(seq):
            ends = [v[v.shape[0] - 8:, t] for v in seq[:2] for t in (lo, hi)]
            anchors = {0: seq[0][0:8, lo]}
            anchors.update(zip(cfg["AG"], ends))
            mac(P, s + 1, anchors)

        x2 = mlp(_unpack(xn_ref[...]), ug_ref[X1], side1, None)
        inv_dot()
        xn3, old = mid_norm(x2)
        side2 = lambda seq: side_post(old, qb.at[n1], kb.at[n2], vb.at[n2], paced(seq, 2 * NU, *cfg["SP"]))
        emit(mlp(xn3, zeros(), side2, X3), s)

    @pl.when(s == NB - 1)
    def _():
        xn = _unpack(xn_ref[...])
        act(gu(0, xn), starts[0])
        act(gu(1, xn), starts[1])
        acc = dn(0, ug_ref[X1])
        act(gu(3, xn), starts[3])
        act(gu(2, xn), starts[2])
        xn3, old = mid_norm(dn(2, dn(3, dn(1, acc))))

        def side3(seq):
            anchors = paced(seq, NU, 1000, 128)
            for g in range(NU):
                rs = slice(g * UR, (g + 1) * UR)
                ug_ref[FENCE, 8:16, lo] = anchors[g]
                x = ug_ref[X2 + zd, rs, :]
                ug_ref[X3, rs, :] = x + (x - old[0]) * old[1] * ug_ref[YY + zd, rs, :]

        emit(mlp(xn3, zeros(), side3, X3), NB - 1)
        wait(*[out_copy(b) for b in range(NB)])


_CFG = dict(JG=4, AG=(6, 10, 14), HOLD=128, DR=128,
            SP=(1000, 64, 5700, 72), FP=(64, 96, 4300, 110), NZ=8)


@jax.jit
def pallas_interleave_layers__ssm_conv_h3__geglu_ffn__prompt_kernel(
        A_q, A_k, A_v, A_shift_k, A_ssm_k, A_ssm_D, B_x, B_w_gate, B_w_up, B_w_down):
    _, S, D = A_q.shape
    F = B_w_gate.shape[1]
    KS = A_shift_k.shape[1]
    NB = S // TM
    P = S // B
    CH = (512, 512, 512, 256)
    assert sum(CH) == F and S % TM == 0 and NB >= 4 and D % 64 == 0 and KS == 4
    ft, fi = _dft_tables()
    to_ds = lambda x: jnp.swapaxes(x, 1, 2).reshape(D, S)
    hbm = pl.BlockSpec(memory_space=pl.ANY)
    blocks = pltpu.VMEM((NB, D, TM), BF16)
    out_t = pl.pallas_call(
        functools.partial(_kernel, D=D, F=F, NB=NB, KS=KS, CH=CH, cfg=_CFG),
        out_shape=jax.ShapeDtypeStruct((D, S), A_q.dtype),
        grid=(NB,),
        in_specs=[hbm] * 11,
        out_specs=hbm,
        scratch_shapes=[
            blocks,
            pltpu.VMEM((3 * P - 1 - 2 * PB + 12, D, 2 * B), F32),
            pltpu.VMEM((D // 2, TM), U32),
            pltpu.VMEM((D // 2, PB * 2 * B), U32),
            pltpu.VMEM((D // 2, TM), U32),
            pltpu.VMEM((32, TM), F32),
            pltpu.VMEM((F, D), U32),
            pltpu.VMEM((D // 2, F), U32),
            pltpu.VMEM((D // 2, B), U32),
            pltpu.VMEM((F // 2, TM), U32),
            blocks, blocks, blocks, blocks,
            pltpu.VMEM((KS, D), BF16),
            pltpu.VMEM((D,), BF16),
            pltpu.VMEM((B // 2, 2 * B), U32),
            pltpu.VMEM((B, B), U32),
            pltpu.VMEM((D, F), BF16),
            pltpu.VMEM((D, F), BF16),
            pltpu.VMEM((D, F), BF16),
            pltpu.SemaphoreType.DMA((4 + 3 * len(CH) + 5 * NB,)),
        ],
        compiler_params=pltpu.CompilerParams(vmem_limit_bytes=100 * 2**20,
                                             dimension_semantics=("arbitrary",)),
    )(to_ds(A_q), to_ds(A_k), to_ds(A_v), A_ssm_k, A_shift_k.T, A_ssm_D,
      jnp.asarray(ft), jnp.asarray(fi), B_w_gate, B_w_up, B_w_down.T)
    return jnp.swapaxes(out_t.reshape(1, D, S), 1, 2)
```
